```python
import jax
import jax.numpy as jnp

def _softmax(x, axis=-1):
    return jax.nn.softmax(x, axis=axis)

def _gelu(x):
    return jax.nn.gelu(x, approximate=True)

def _silu(x):
    return jax.nn.silu(x)

def _sigmoid(x):
    return jax.nn.sigmoid(x)

def _layernorm(x, axis=-1, eps=1e-05):
    m = jnp.mean(x, axis=axis, keepdims=True)
    v = jnp.var(x, axis=axis, keepdims=True)
    return (x - m) / jnp.sqrt(v + eps)

def _scatter_add(tgt, idx, src, axis=0):
    return tgt.at[idx].add(src)

def _segment_sum(src, seg, n):
    return jax.ops.segment_sum(src, seg, n)

class _Rng:

    def __init__(self, key):
        self._k = key

    def _next(self):
        self._k, sub = jax.random.split(self._k)
        return sub

    def normal(self, shape):
        return jax.random.normal(self._next(), shape, dtype=jnp.bfloat16)

    def randint(self, lo, hi, shape):
        return jax.random.randint(self._next(), shape, lo, hi, dtype=jnp.int32)

    def uniform(self, shape, lo=0.0, hi=1.0):
        return jax.random.uniform(self._next(), shape, jnp.bfloat16, lo, hi)

    def permutation(self, n):
        return jax.random.permutation(self._next(), n)
kernel_name = 'interleave_layers__memory_aug_recurrent_mem_tr__moe_arch_mod__prompt'

def setup_inputs():
    _rng = _Rng(jax.random.key(int.from_bytes(__import__("os").urandom(4), "little")))
    _w = lambda a: (lambda t: t.astype(jnp.bfloat16) if jnp.issubdtype(t.dtype, jnp.floating) else t)(jnp.asarray(a))

    def _A_setup():
        B, S, Dm = (1, 2048, 512)
        H, Dh = (32, 128)
        M, seg = (8, 32)
        seg = min(seg, S)
        S = S // seg * seg
        return {'x': _w((lambda *s: _rng.normal(s) * 0.05)(B, S, Dm)), 'mem0': _w((lambda *s: _rng.normal(s) * 0.05)(B, M, Dm)), 'Wq': _w((lambda *s: _rng.normal(s) * 0.05)(Dm, H, Dh) * Dm ** (-0.5)), 'Wk': _w((lambda *s: _rng.normal(s) * 0.05)(Dm, H, Dh) * Dm ** (-0.5)), 'Wv': _w((lambda *s: _rng.normal(s) * 0.05)(Dm, H, Dh) * Dm ** (-0.5)), 'Wo': _w((lambda *s: _rng.normal(s) * 0.05)(H, Dh, Dm) * (H * Dh) ** (-0.5)), 'seg_len': seg}
    _A_in = _A_setup()

    def _B_setup():
        B, S, D, F, C = (1, 2048, 512, 1792, 1)
        return {'x': _w((lambda *s: _rng.normal(s) * 0.05)(B, S, D)), 'w_r': _w((lambda *s: _rng.normal(s) * 0.05)(D)), 'w_gate': _w((lambda *s: _rng.normal(s) * 0.05)(D, F)), 'w_up': _w((lambda *s: _rng.normal(s) * 0.05)(D, F)), 'w_down': _w((lambda *s: _rng.normal(s) * 0.05)(F, D))}
    _B_in = _B_setup()
    return {'A_x': _A_in['x'], 'A_mem0': _A_in['mem0'], 'A_Wq': _A_in['Wq'], 'A_Wk': _A_in['Wk'], 'A_Wv': _A_in['Wv'], 'A_Wo': _A_in['Wo'], 'A_seg_len': _A_in['seg_len'], 'B_x': _B_in['x'], 'B_w_r': _B_in['w_r'], 'B_w_gate': _B_in['w_gate'], 'B_w_up': _B_in['w_up'], 'B_w_down': _B_in['w_down']}

def reference(A_x, A_mem0, A_Wq, A_Wk, A_Wv, A_Wo, A_seg_len, B_x, B_w_r, B_w_gate, B_w_up, B_w_down):

    def _A_ref(x, mem0, Wq, Wk, Wv, Wo, seg_len):
        B, S, Dm = x.shape
        H, Dh = (Wq.shape[1], Wq.shape[2])
        M = mem0.shape[1]
        scale = Dh ** (-0.5)
        n_seg = S // seg_len
        L = M + seg_len
        idx = jnp.arange(L)
        mask = (idx[:, None] < M) | (idx[:, None] >= idx[None, :])
        mem = mem0
        outs = []
        for s in range(n_seg):
            xs = x[:, s * seg_len:(s + 1) * seg_len, :].copy()
            h = jnp.concatenate([mem, xs], axis=1)
            q = jnp.einsum('btd,dhe->bhte', h, Wq)
            k = jnp.einsum('btd,dhe->bhte', h, Wk)
            v = jnp.einsum('btd,dhe->bhte', h, Wv)
            scores = jnp.einsum('bhqe,bhke->bhqk', q, k) * scale
            scores = jnp.where(mask[None, None], scores, -1000000000.0)
            p = _softmax(scores, axis=-1)
            o = jnp.einsum('bhqk,bhke->bhqe', p, v)
            o = jnp.einsum('bhte,hed->btd', o, Wo)
            mem = o[:, :M, :].copy()
            outs.append(o[:, M:, :])
        return jnp.concatenate(outs, axis=1)

    def _B_ref(x, w_r, w_gate, w_up, w_down):
        B, S, D = x.shape
        C = 1
        r = x @ w_r
        idx = jnp.argsort(-r, axis=-1)[:, :C]
        idx_e = jnp.repeat(idx.reshape(B, C, 1), D, axis=2)
        x_sel = jnp.take_along_axis(x, idx_e, axis=1)
        g = _silu(x_sel @ w_gate)
        u = x_sel @ w_up
        y = g * u @ w_down
        r_sel = _sigmoid(jnp.take_along_axis(r, idx, axis=1))
        y = y * r_sel.reshape(B, C, 1)
        b_off = (jnp.arange(B) * S).reshape(B, 1)
        flat_idx = (idx + b_off).reshape(B * C)
        zero = (x * 0.0).reshape(B * S, D)
        upd = _scatter_add(zero, flat_idx, y.reshape(B * C, D), axis=0)
        return x + upd.reshape(B, S, D)
    x = A_x
    x = x + _A_ref(_layernorm(x, axis=-1), A_mem0, A_Wq, A_Wk, A_Wv, A_Wo, A_seg_len)
    x = x + _B_ref(_layernorm(x, axis=-1), B_w_r, B_w_gate, B_w_up, B_w_down)
    x = x + _A_ref(_layernorm(x, axis=-1), A_mem0, A_Wq, A_Wk, A_Wv, A_Wo, A_seg_len)
    x = x + _B_ref(_layernorm(x, axis=-1), B_w_r, B_w_gate, B_w_up, B_w_down)
    return x
```

```python
import functools

import jax
import jax.numpy as jnp
import numpy as np
from jax import lax
import jax.experimental.pallas as pl
import jax.experimental.pallas.tpu as pltpu

F32 = jnp.float32
BF16 = jnp.bfloat16
LANES = 128
N_LAYERS = 2
PAIRS_PER_GROUP = 4


def _mm(a, b):
    return lax.dot_general(a, b, (((1,), (0,)), ((), ())), preferred_element_type=F32)


def _mm_nt(a, b):
    return lax.dot_general(a, b, (((1,), (1,)), ((), ())), preferred_element_type=F32)


def _rb(x):
    return x.astype(BF16).astype(F32)


def _layernorm(x):
    inv_d = 1.0 / x.shape[-1]
    mean = jnp.sum(x, axis=-1, keepdims=True) * inv_d
    cen = x - mean
    var = jnp.sum(cen * cen, axis=-1, keepdims=True) * inv_d
    eps = float(np.asarray(1e-5, dtype=BF16))
    std = _rb(jnp.sqrt(_rb(_rb(var) + eps)))
    return _rb(_rb(x - _rb(mean)) * (1.0 / std))


def _kernel(x_hbm, mem0_ref, wq_hbm, wk_hbm, wv_hbm, wo_hbm, wr_ref, wg_hbm, wu_hbm, wd_hbm,
            out_hbm,
            raw, wq, wk, wv, wo, wg, wu, wd, xres, x1buf, hbuf, obuf, sems,
            *, seg, n_seg, n_heads):
    d_model = x_hbm.shape[1]
    n_mem = mem0_ref.shape[0]
    dh = wq.shape[2]
    rows = n_mem + seg
    n_pairs = n_heads // 2
    n_groups = n_pairs // PAIRS_PER_GROUP
    n_col = d_model // LANES
    scale = dh ** -0.5

    x_copy = pltpu.make_async_copy(x_hbm, xres.at[pl.ds(seg, n_seg * seg)], sems.at[0])
    qkv_copies = [pltpu.make_async_copy(src.bitcast(jnp.uint32), raw.at[i], sems.at[1 + i])
                  for i, src in enumerate((wq_hbm, wk_hbm, wv_hbm))]
    wo_copies = [pltpu.make_async_copy(wo_hbm.at[:, pl.ds(n * LANES, LANES)], wo.at[n], sems.at[4 + n])
                 for n in range(n_col)]
    mlp_copies = [pltpu.make_async_copy(src, dst, sems.at[4 + n_col + i])
                  for i, (src, dst) in enumerate(((wg_hbm, wg), (wu_hbm, wu), (wd_hbm, wd)))]
    for c in qkv_copies + wo_copies + [x_copy]:
        c.start()

    zeros = jnp.zeros((seg, d_model), BF16)
    xres[pl.ds(0, seg), :] = zeros
    xres[pl.ds((n_seg + 1) * seg, seg), :] = zeros
    obuf[...] = jnp.zeros(obuf.shape, F32)

    for i, dst in enumerate((wq, wk, wv)):
        qkv_copies[i].wait()

        def split_pair(p, carry, i=i, dst=dst):
            w = raw[i, pl.ds(p, d_model, stride=n_pairs), :]
            dst[2 * p] = pltpu.bitcast(w << 16, F32).astype(BF16)
            dst[2 * p + 1] = pltpu.bitcast(w & np.uint32(0xFFFF0000), F32).astype(BF16)
            return carry

        lax.fori_loop(0, n_pairs, split_pair, 0)
    for c in wo_copies:
        c.wait()
    x_copy.wait()
    for c in mlp_copies:
        c.start()

    r = lax.broadcasted_iota(jnp.int32, (2 * rows, 2 * rows), 0)
    c = lax.broadcasted_iota(jnp.int32, (2 * rows, 2 * rows), 1)
    r_hi, c_hi = r >= rows, c >= rows
    ri = jnp.where(r_hi, r - rows, r)
    ci = jnp.where(c_hi, c - rows, c)
    same_head = r_hi == c_hi
    visible = same_head & ((ri < n_mem) | (ri >= ci))
    fill = jnp.where(same_head, -1e9 / scale, -np.inf).astype(F32)
    exp2_scale = float(scale * np.log2(np.e))
    w_r = wr_ref[...].astype(F32)
    sub = lax.broadcasted_iota(jnp.int32, (8, 1), 0)

    def slot(i):
        return pl.ds(pl.multiple_of(i * seg, seg), seg)

    def attention(h):
        q, k, v, e, inv, o = {}, {}, {}, {}, {}, {}
        acc = [None] * n_col

        def pairs(g):
            return range(g * PAIRS_PER_GROUP, (g + 1) * PAIRS_PER_GROUP)

        def project(w, p):
            return jnp.concatenate([_mm(h, w[2 * p]), _mm(h, w[2 * p + 1])], axis=0)

        def qk_proj(g):
            for p in pairs(g):
                q[p] = project(wq, p)
                k[p] = project(wk, p).astype(BF16)

        def v_proj(g):
            for p in pairs(g):
                v[p] = project(wv, p).astype(BF16)

        def scores(g):
            for p in pairs(g):
                s = jnp.where(visible, _mm_nt(q[p], k[p]), fill)
                e[p] = jnp.exp2((s - jnp.max(s, axis=1, keepdims=True)) * exp2_scale)
                l = jnp.sum(e[p], axis=1, keepdims=True)
                r0 = pl.reciprocal(l, approx=True)
                inv[p] = r0 * (2.0 - l * r0)

        def mix(g):
            for p in pairs(g):
                o[p] = _mm(e[p], v[p]) * inv[p]

        def out_proj(g):
            lhs = jnp.concatenate(
                [o[p][j * rows:(j + 1) * rows] for p in pairs(g) for j in range(2)], axis=1)
            width = lhs.shape[1]
            for n in range(n_col):
                t = _mm(lhs, wo[n, pl.ds(g * width, width), :])
                acc[n] = t if acc[n] is None else acc[n] + t

        qk_proj(0)
        for g in range(1, n_groups):
            qk_proj(g)
            scores(g - 1)
        v_proj(0)
        scores(n_groups - 1)
        for g in range(1, n_groups):
            v_proj(g)
            mix(g - 1)
        out_proj(0)
        mix(n_groups - 1)
        for g in range(1, n_groups):
            out_proj(g)
        return jnp.concatenate(acc, axis=1)

    def finish_rows(i, best, best_row):
        x1 = _rb(xres[slot(i), :].astype(F32) + _rb(obuf[...]))
        x1buf[slot(i), :] = x1.astype(BF16)
        n1 = _layernorm(x1)
        xres[slot(i), :] = (x1 + n1).astype(BF16)
        score = _rb(jnp.sum(n1 * w_r, axis=-1, keepdims=True))
        score = jnp.where(i > 0, score, -np.inf)
        for j in range(seg // 8):
            sj = score[8 * j:8 * j + 8]
            better = sj > best
            best = jnp.where(better, sj, best)
            best_row = jnp.where(better, i * seg + 8 * j + sub, best_row)
        return best, best_row

    def step(s, carry):
        mem, best, best_row = carry
        h = jnp.concatenate([mem, hbuf[...]], axis=0)
        best, best_row = finish_rows(s, best, best_row)
        nxt = _layernorm(xres[slot(s + 2), :].astype(F32))
        out = attention(h)
        hbuf[...] = nxt
        obuf[...] = out[n_mem:]
        return out[:n_mem], best, best_row

    def layer(l, carry):
        hbuf[...] = _layernorm(xres[pl.ds(seg, seg), :].astype(F32))
        init = (mem0_ref[...].astype(F32),
                jnp.full((8, 1), -np.inf, F32),
                jnp.full((8, 1), seg, jnp.int32))
        _, best, best_row = lax.fori_loop(0, n_seg, step, init)
        best, best_row = finish_rows(n_seg, best, best_row)

        @pl.when(l == 0)
        def _():
            for cp in mlp_copies:
                cp.wait()

        top = jnp.max(best, axis=0, keepdims=True)
        row = jnp.min(jnp.where(best == top, best_row, (n_seg + 1) * seg - 1).astype(F32))
        row = jnp.clip(row.astype(jnp.int32), seg, (n_seg + 1) * seg - 1)
        blk = pl.ds(pl.multiple_of((row // 16) * 16, 16), 16)
        x1 = x1buf[blk, :].astype(F32)
        n1 = _layernorm(x1)
        score = _rb(jnp.sum(n1 * w_r, axis=-1, keepdims=True))
        xs = n1.astype(BF16)
        gate = _rb(_mm(xs, wg[...]))
        gate = _rb(gate * _rb(jax.nn.sigmoid(gate)))
        up = _rb(_mm(xs, wu[...]))
        y = _rb(_mm((gate * up).astype(BF16), wd[...]))
        y = _rb(y * _rb(jax.nn.sigmoid(score)))
        chosen = lax.broadcasted_iota(jnp.int32, (16, 1), 0) == row % 16
        xres[blk, :] = (x1 + _rb(n1 + jnp.where(chosen, y, 0.0))).astype(BF16)
        return carry

    lax.fori_loop(0, N_LAYERS, layer, 0)

    out_copy = pltpu.make_async_copy(xres.at[pl.ds(seg, n_seg * seg)], out_hbm, sems.at[0])
    out_copy.start()
    out_copy.wait()


def pallas_interleave_layers__memory_aug_recurrent_mem_tr__moe_arch_mod__prompt_kernel(
    A_x, A_mem0, A_Wq, A_Wk, A_Wv, A_Wo, A_seg_len, B_x, B_w_r, B_w_gate, B_w_up, B_w_down,
):
    del B_x
    batch, seq, d_model = A_x.shape
    assert batch == 1
    n_heads, dh = A_Wq.shape[1:]
    n_mem = A_mem0.shape[1]
    seg = int(A_seg_len)
    n_seg = seq // seg
    d_ff = B_w_gate.shape[1]

    any_spec = pl.BlockSpec(memory_space=pl.ANY)
    vmem_spec = pl.BlockSpec(memory_space=pltpu.VMEM)
    padded = (n_seg + 2) * seg
    out = pl.pallas_call(
        functools.partial(_kernel, seg=seg, n_seg=n_seg, n_heads=n_heads),
        out_shape=jax.ShapeDtypeStruct((seq, d_model), A_x.dtype),
        in_specs=[any_spec, vmem_spec, any_spec, any_spec, any_spec, any_spec,
                  vmem_spec, any_spec, any_spec, any_spec],
        out_specs=any_spec,
        scratch_shapes=[
            pltpu.VMEM((3, d_model * n_heads // 2, dh), jnp.uint32),
            pltpu.VMEM((n_heads, d_model, dh), BF16),
            pltpu.VMEM((n_heads, d_model, dh), BF16),
            pltpu.VMEM((n_heads, d_model, dh), BF16),
            pltpu.VMEM((d_model // LANES, n_heads * dh, LANES), BF16),
            pltpu.VMEM((d_model, d_ff), BF16),
            pltpu.VMEM((d_model, d_ff), BF16),
            pltpu.VMEM((d_ff, d_model), BF16),
            pltpu.VMEM((padded, d_model), BF16),
            pltpu.VMEM((padded, d_model), BF16),
            pltpu.VMEM((seg, d_model), F32),
            pltpu.VMEM((seg, d_model), F32),
            pltpu.SemaphoreType.DMA((7 + d_model // LANES,)),
        ],
        compiler_params=pltpu.CompilerParams(vmem_limit_bytes=100 * 1024 * 1024),
    )(
        A_x.reshape(seq, d_model),
        A_mem0.reshape(n_mem, d_model),
        A_Wq.reshape(d_model * n_heads, dh),
        A_Wk.reshape(d_model * n_heads, dh),
        A_Wv.reshape(d_model * n_heads, dh),
        A_Wo.reshape(n_heads * dh, d_model),
        B_w_r.reshape(1, d_model),
        B_w_gate,
        B_w_up,
        B_w_down,
    )
    return out.reshape(batch, seq, d_model)
```

```python
import jax
import jax.numpy as jnp
import numpy as np
from jax import lax
import jax.experimental.pallas as pl
import jax.experimental.pallas.tpu as pltpu
CFG = dict(qplan=[[0,16,4]], u0=4, u1=4, n0=64, n1=64, order0="F", order1="D", flags={}, newton=1, ksplit=3, pu=4, xch=4, stop=0, brows=8, nochk=1)
CFG.update({'qplan': [[0, 1, 1], [1, 4, 3], [4, 16, 6]]})

F32 = jnp.float32
BF16 = jnp.bfloat16
U32 = jnp.uint32
LANES = 128
SUB = 8
PAIRS_PER_GROUP = 4


def _mm(a, b):
    return lax.dot_general(a, b, (((1,), (0,)), ((), ())), preferred_element_type=F32)


def _mm_nt(a, b):
    return lax.dot_general(a, b, (((1,), (1,)), ((), ())), preferred_element_type=F32)


def _rb(x):
    return x.astype(BF16).astype(F32)


def _w(words):
    return pltpu.bitcast(words, BF16)


def _layernorm(x):
    inv_d = 1.0 / x.shape[-1]
    mean = jnp.sum(x, axis=-1, keepdims=True) * inv_d
    cen = x - mean
    var = jnp.sum(cen * cen, axis=-1, keepdims=True) * inv_d
    eps = float(np.asarray(1e-5, dtype=BF16))
    std = _rb(jnp.sqrt(_rb(_rb(var) + eps)))
    return _rb(_rb(x - _rb(mean)) * (1.0 / std))


def _kernel(x_hbm, mem0_hbm, wq_hbm, wk_hbm, wv_hbm, wo_hbm, wr_hbm, wg_hbm, wu_hbm, wd_hbm,
            out_hbm,
            raw, wq, wk, wv, wo, wg, wu, wd, mem0, wr, xres, x1buf, xtail, ntail, qpre, kpre, hbuf, obuf, fixbuf,
            sems):
    n_seg, seg, d_model = x_hbm.shape
    n_mem = mem0.shape[0]
    n_heads, _, dh = wq.shape
    rows = n_mem + seg
    n_pairs = n_heads // 2
    n_groups = n_pairs // PAIRS_PER_GROUP
    n_col = d_model // LANES
    scale = dh ** -0.5
    head = seg - SUB
    xch = CFG["xch"]
    first = 16
    PU = CFG["pu"]

    sem_ids = iter(range(3 * n_pairs, sems.shape[0]))

    def copy(src, dst):
        return pltpu.make_async_copy(src, dst, sems.at[next(sem_ids)])

    per = n_seg // xch
    tail_copies = [copy(x_hbm.at[pl.ds(j * per, per), pl.ds(head, SUB), :], xtail.at[pl.ds(j * per, per)])
                   for j in range(xch)]

    def pair_copy(i, p):
        src = (wq_hbm, wk_hbm, wv_hbm)[i].bitcast(U32)
        return pltpu.make_async_copy(src.at[:, p, :], raw.at[i * n_pairs + p], sems.at[i * n_pairs + p])

    early = [copy(mem0_hbm, mem0), copy(wr_hbm, wr), copy(x_hbm.at[pl.ds(0, first)], xres.at[pl.ds(1, first)])]
    early += [copy(wo_hbm.bitcast(U32).at[:, pl.ds(n * LANES, LANES)], wo.at[n]) for n in range(n_col)]
    x_rest = copy(x_hbm.at[pl.ds(first, n_seg - first)], xres.at[pl.ds(1 + first, n_seg - first)])
    mlp_copies = [copy(src.bitcast(U32), dst) for src, dst in ((wg_hbm, wg), (wu_hbm, wu), (wd_hbm, wd))]
    out_sem = sems.at[next(sem_ids)]
    for c in tail_copies:
        c.start()
    for p in range(n_pairs):
        pair_copy(0, p).start()
    for p in range(n_pairs):
        pair_copy(1, p).start()
        pair_copy(2, p).start()
    for c in early + ([] if CFG["stop"] else [x_rest] + mlp_copies):
        c.start()

    zeros = jnp.zeros((seg, d_model), BF16)
    xres[0] = zeros
    xres[n_seg + 1] = zeros
    obuf[...] = jnp.zeros(obuf.shape, F32)

    for j in range(xch):
        tail_copies[j].wait()
        t = xtail[pl.ds(j * per, per)].astype(F32).reshape(per * SUB, d_model)
        ntail[pl.ds(j * per * SUB // 2, per * SUB // 2), :] = pltpu.bitcast(_layernorm(t).astype(BF16), U32)

    def split(i, p):
        even = raw[i * n_pairs + p, pl.ds(0, d_model // 2, stride=2), :]
        odd = raw[i * n_pairs + p, pl.ds(1, d_model // 2, stride=2), :]
        halves = ((even & np.uint32(0xFFFF)) | (odd << 16), (even >> 16) | (odd & np.uint32(0xFFFF0000)))
        for j, half in enumerate(halves):
            (wq, wk, wv)[i][2 * p + j] = half
            if i < 2:
                (qpre, kpre)[i][2 * p + j] = _mm(_w(ntail[...]), _w(half))

    def load_pairs(which, lo, hi, unroll):
        def body(it, carry):
            ps = [lo + it * unroll + u for u in range(unroll)]
            for p in ps:
                for i in which:
                    pair_copy(i, p).wait()
            for p in ps:
                for i in which:
                    split(i, p)
            return carry
        if hi - lo == unroll:
            body(0, 0)
        else:
            lax.fori_loop(0, (hi - lo) // unroll, body, 0)

    for lo, hi, unroll in CFG["qplan"]:
        load_pairs((0,), lo, hi, unroll)
    load_pairs((1, 2), 0, n_pairs, PU)
    for c in early:
        c.wait()
    if CFG["stop"]:
        return

    r = lax.broadcasted_iota(jnp.int32, (2 * rows, 2 * rows), 0)
    c = lax.broadcasted_iota(jnp.int32, (2 * rows, 2 * rows), 1)
    r_hi, c_hi = r >= rows, c >= rows
    ri = jnp.where(r_hi, r - rows, r)
    ci = jnp.where(c_hi, c - rows, c)
    same_head = r_hi == c_hi
    visible = same_head & ((ri < n_mem) | (ri >= ci))
    fill = jnp.where(same_head, -1e9 / scale, -np.inf).astype(F32)
    exp2_scale = float(scale * np.log2(np.e))
    w_r = wr[...].astype(F32).reshape(1, d_model)
    sub = lax.broadcasted_iota(jnp.int32, (SUB, 1), 0)

    def attention(mem, tok, pre_rows, side, order):
        q, k, v, e, inv, o = {}, {}, {}, {}, {}, {}
        acc = [None] * n_col
        h = jnp.concatenate([tok, mem], axis=0)
        qp, kp = (None, None) if pre_rows is None else (qpre, kpre)

        def pairs(g):
            return range(g * PAIRS_PER_GROUP, (g + 1) * PAIRS_PER_GROUP)

        def lhs_for(pre):
            return h if pre is None else jnp.concatenate([h[:head], h[seg:]], axis=0)

        def arrange(t, pre, hd):
            if pre is None:
                return [t[seg:], t[:seg]]
            return [t[head:], t[:head], pre[hd, pre_rows, :]]

        def project(w, pre, hd):
            return arrange(_mm(lhs_for(pre), _w(w[hd])), pre, hd)

        def cat(parts):
            return jnp.concatenate(parts, axis=0)

        def first_pair():
            cut = CFG["ksplit"] * LANES
            lhs = lhs_for(qp)
            ws = [wq.at[0], wq.at[1], wk.at[0], wk.at[1]]
            lo = jnp.concatenate([_w(w[:cut // 2, :]) for w in ws], axis=1)
            hi = jnp.concatenate([_w(w[cut // 2:, :]) for w in ws], axis=1)
            t = _mm(lhs[:, :cut], lo)
            t = _mm(lhs[:, cut:], hi) + t
            ts = [t[:, j * dh:(j + 1) * dh] for j in range(4)]
            q[0] = cat(arrange(ts[0], qp, 0) + arrange(ts[1], qp, 1))
            k[0] = cat(arrange(ts[2], kp, 0) + arrange(ts[3], kp, 1)).astype(BF16)

        def QK(g):
            for p in pairs(g):
                if p == 0:
                    first_pair()
                    continue
                q[p] = cat(project(wq, qp, 2 * p) + project(wq, qp, 2 * p + 1))
                k[p] = cat(project(wk, kp, 2 * p) + project(wk, kp, 2 * p + 1)).astype(BF16)

        def V(g):
            for p in pairs(g):
                v[p] = cat(project(wv, None, 2 * p) + project(wv, None, 2 * p + 1)).astype(BF16)

        def QVK(g):
            for p in pairs(g):
                if p == 0:
                    first_pair()
                    v[p] = cat(project(wv, None, 2 * p) + project(wv, None, 2 * p + 1)).astype(BF16)
                    continue
                qs, ks, vs = [], [], []
                for hd in (2 * p, 2 * p + 1):
                    qs += project(wq, qp, hd)
                    vs += project(wv, None, hd)
                    ks += project(wk, kp, hd)
                q[p], k[p], v[p] = cat(qs), cat(ks).astype(BF16), cat(vs).astype(BF16)

        def S(g):
            for p in pairs(g):
                s = jnp.where(visible, _mm_nt(q[p], k[p]), fill)
                e[p] = jnp.exp2((s - jnp.max(s, axis=1, keepdims=True)) * exp2_scale)
                l = jnp.sum(e[p], axis=1, keepdims=True)
                r0 = pl.reciprocal(l, approx=True)
                inv[p] = r0 * (2.0 - l * r0) if CFG["newton"] else r0

        def P(g):
            for p in pairs(g):
                o[p] = _mm(e[p], v[p]) * inv[p]

        def O(g):
            lhs = jnp.concatenate(
                [o[p][j * rows:(j + 1) * rows] for p in pairs(g) for j in range(2)], axis=1)
            width = lhs.shape[1] // 2
            for n in range(n_col):
                t = _mm(lhs, _w(wo[n, pl.ds(g * width, width), :]))
                acc[n] = t if acc[n] is None else acc[n] + t

        def tie(i):
            nonlocal h
            never = side[i]()
            first8 = jnp.where(never, 0.0, h[:SUB, :LANES])
            top = jnp.concatenate([first8, h[:SUB, LANES:]], axis=1)
            h = jnp.concatenate([top, h[SUB:]], axis=0)

        fns = dict(T=tie, A=QK, C=QVK, V=V, S=S, P=P, O=O, X=lambda i: side[i]())
        orders = dict(
            D="X1 A0 A1 T0 S0 A2 S1 A3 S2 V0 S3 V1 P0 V2 P1 V3 P2 O0 O1 P3 O2 O3",
            F="X1 C0 T0 C1 S0 C2 S1 P0 C3 P1 S2 S3 O0 O1 P2 P3 O2 O3",
        )
        for t in orders.get(order, order).split():
            fns[t[0]](int(t[1]))
        return jnp.concatenate(acc, axis=1)

    def finish_rows(i, o_tok, best, best_row):
        x1 = _rb(xres[i].astype(F32) + _rb(o_tok))
        x1buf[i] = x1.astype(BF16)
        n1 = _layernorm(x1)
        xres[i] = (x1 + n1).astype(BF16)
        score = _rb(jnp.sum(n1 * w_r, axis=-1, keepdims=True))
        score = jnp.where(i > 0, score, -np.inf)
        for j in range(seg // SUB):
            sj = score[SUB * j:SUB * (j + 1)]
            better = sj > best
            best = jnp.where(better, sj, best)
            best_row = jnp.where(better, (i - 1) * seg + SUB * j + sub, best_row)
        return best, best_row

    def attention_layer(first_layer):
        U = CFG["u0"] if first_layer else CFG["u1"]
        order = CFG["order0"] if first_layer else CFG["order1"]

        def step(it, carry):
            mem, best, best_row = carry
            if first_layer:
                @pl.when(it == 1)
                def _():
                    x_rest.wait()
            else:
                @pl.when(it > 1)
                def _():
                    lo = (it - 2) * U
                    pltpu.make_async_copy(xres.at[pl.ds(lo + 1, U)], out_hbm.at[pl.ds(lo, U)], out_sem).start()
            st = dict(best=best, best_row=best_row, tok=hbuf[...], o=obuf[...])
            for u in range(U):
                s = it * U + u
                def fin(s=s):
                    st["best"], st["best_row"] = finish_rows(s, st["o"], st["best"], st["best_row"])
                    return st["best_row"] < 0
                def nxt(s=s):
                    st["nxt"] = _layernorm(xres[s + 2].astype(F32))
                pre_rows = pl.ds(pl.multiple_of(s * SUB, SUB), SUB) if first_layer else None
                out = attention(mem, st["tok"], pre_rows, (fin, nxt), order)
                mem = out[:n_mem]
                st["tok"] = st["nxt"]; st["o"] = out[n_mem:]
            hbuf[...] = st["tok"]
            obuf[...] = st["o"]
            return mem, st["best"], st["best_row"]

        hbuf[...] = _layernorm(xres[1].astype(F32))
        init = (mem0[...].astype(F32),
                jnp.full((SUB, 1), -np.inf, F32),
                jnp.zeros((SUB, 1), jnp.int32))
        _, best, best_row = lax.fori_loop(0, (CFG["n0"] if first_layer else CFG["n1"]) // U, step, init)
        return finish_rows(n_seg, obuf[...], best, best_row)

    BR = CFG["brows"]

    def routed_update(best, best_row):
        top = jnp.max(best, axis=0, keepdims=True)
        row = jnp.min(jnp.where(best == top, best_row, n_seg * seg - 1).astype(F32))
        row = jnp.clip(row.astype(jnp.int32), 0, n_seg * seg - 1)
        s = row // seg
        blk = pl.ds(pl.multiple_of(row % seg // BR * BR, BR), BR)
        x1 = x1buf[s + 1, blk, :].astype(F32)
        n1 = _layernorm(x1)
        score = _rb(jnp.sum(n1 * w_r, axis=-1, keepdims=True))
        gate = _rb(_mm(n1, _w(wg[...])))
        gate = _rb(gate * _rb(jax.nn.sigmoid(gate)))
        up = _rb(_mm(n1, _w(wu[...])))
        y = _rb(_mm(_rb(gate * up), _w(wd[...])))
        y = _rb(y * _rb(jax.nn.sigmoid(score)))
        chosen = lax.broadcasted_iota(jnp.int32, (BR, 1), 0) == row % BR
        return s, blk, (x1 + _rb(n1 + jnp.where(chosen, y, 0.0))).astype(BF16)

    best, best_row = attention_layer(True)
    for cp in mlp_copies:
        cp.wait()
    s, blk, new = routed_update(best, best_row)
    xres[s + 1, blk, :] = new

    best, best_row = attention_layer(False)
    lo = CFG["n1"] - 2 * CFG["u1"]
    pltpu.make_async_copy(xres.at[pl.ds(lo + 1, n_seg - lo)], out_hbm.at[pl.ds(lo, n_seg - lo)], out_sem).start()
    s, blk, new = routed_update(best, best_row)
    fixbuf[...] = new
    pltpu.make_async_copy(xres.at[pl.ds(1, n_seg)], out_hbm, out_sem).wait()
    fix = pltpu.make_async_copy(fixbuf, out_hbm.at[s, blk, :], out_sem)
    fix.start()
    fix.wait()


def pallas_interleave_layers__memory_aug_recurrent_mem_tr__moe_arch_mod__prompt_kernel(
    A_x, A_mem0, A_Wq, A_Wk, A_Wv, A_Wo, A_seg_len, B_x, B_w_r, B_w_gate, B_w_up, B_w_down,
):
    del B_x
    batch, seq, d_model = A_x.shape
    assert batch == 1
    n_heads, dh = A_Wq.shape[1:]
    n_mem = A_mem0.shape[1]
    seg = int(A_seg_len)
    n_seg = seq // seg
    d_ff = B_w_gate.shape[1]

    any_spec = pl.BlockSpec(memory_space=pl.ANY)
    out = pl.pallas_call(
        _kernel,
        out_shape=jax.ShapeDtypeStruct((n_seg, seg, d_model), A_x.dtype),
        in_specs=[any_spec] * 10,
        out_specs=any_spec,
        scratch_shapes=[
            pltpu.VMEM((3 * n_heads // 2, d_model, dh), U32),
            pltpu.VMEM((n_heads, d_model // 2, dh), U32),
            pltpu.VMEM((n_heads, d_model // 2, dh), U32),
            pltpu.VMEM((n_heads, d_model // 2, dh), U32),
            pltpu.VMEM((d_model // LANES, n_heads * dh // 2, LANES), U32),
            pltpu.VMEM((d_model // 2, d_ff), U32),
            pltpu.VMEM((d_model // 2, d_ff), U32),
            pltpu.VMEM((d_ff // 2, d_model), U32),
            pltpu.VMEM((n_mem, d_model), BF16),
            pltpu.VMEM((d_model,), BF16),
            pltpu.VMEM((n_seg + 2, seg, d_model), BF16),
            pltpu.VMEM((n_seg + 1, seg, d_model), BF16),
            pltpu.VMEM((n_seg, SUB, d_model), BF16),
            pltpu.VMEM((n_seg * SUB // 2, d_model), U32),
            pltpu.VMEM((n_heads, n_seg * SUB, dh), F32),
            pltpu.VMEM((n_heads, n_seg * SUB, dh), F32),
            pltpu.VMEM((seg, d_model), F32),
            pltpu.VMEM((seg, d_model), F32),
            pltpu.VMEM((CFG["brows"], d_model), BF16),
            pltpu.SemaphoreType.DMA((3 * n_heads // 2 + CFG["xch"] + 8 + d_model // LANES,)),
        ],
        compiler_params=pltpu.CompilerParams(vmem_limit_bytes=100 * 1024 * 1024, flags=CFG["flags"] or None,
            disable_bounds_checks=bool(CFG["nochk"]), disable_semaphore_checks=bool(CFG["nochk"])),
    )(
        A_x.reshape(n_seg, seg, d_model),
        A_mem0.reshape(n_mem, d_model),
        A_Wq,
        A_Wk,
        A_Wv,
        A_Wo.reshape(n_heads * dh, d_model),
        B_w_r,
        B_w_gate,
        B_w_up,
        B_w_down,
    )
    return out.reshape(batch, seq, d_model)
```

```python
import functools
import jax
import jax.numpy as jnp
import numpy as np
from jax import lax
import jax.experimental.pallas as pl
import jax.experimental.pallas.tpu as pltpu
CFG = dict(only=-1, p0={}, p1={}, slag=[2,2,2,4], plag=14, olag=99, ostep=1, stie=0, softlat=450, e_fin=700, e_nxt=750, t_fin=100, t_nxt=0, vlag=4, w0=500, wend=4400, wgap=250, w1lat=0, w2lat=350, tail='S3 P2 O0 O1 P3 O2 O3', nv=1, bc='mem', qplan=[[0,1,1],[1,4,3],[4,16,6]], u0=4, u1=4, n0=64, n1=64, order0="auto", order1="auto", flags={}, newton=1, ksplit=3, pu=4, xch=4, stop=0, brows=8, nochk=1)
CFG.update({'p0': {'w0': 400, 'wend': 3800, 'vlag': 2, 'slag': [3, 3, 3, 3], 'olag': 18, 'tail': 'S3 O0 P2 O1 P3 O2 O3', 'e_fin': 500, 't_fin': 100, 'e_nxt': 1150, 'softlat': 500}, 'p1': {'w0': 300, 'wend': 4000, 'e_nxt': 9000, 'e_fin': 9000, 'wgap': 130, 'tail': 'S3 O0 P2 O1 P3 O2 O3', 't_fin': 260, 'softlat': 700, 'plag': 11}})

F32 = jnp.float32
BF16 = jnp.bfloat16
U32 = jnp.uint32
LANES = 128
SUB = 8
PAIRS_PER_GROUP = 4


def _mm(a, b):
    return lax.dot_general(a, b, (((1,), (0,)), ((), ())), preferred_element_type=F32)


def _mm_nt(a, b):
    return lax.dot_general(a, b, (((1,), (1,)), ((), ())), preferred_element_type=F32)


def _rb(x):
    return x.astype(BF16).astype(F32)


def _w(words):
    return pltpu.bitcast(words, BF16)


def _layernorm(x):
    inv_d = 1.0 / x.shape[-1]
    mean = jnp.sum(x, axis=-1, keepdims=True) * inv_d
    cen = x - mean
    var = jnp.sum(cen * cen, axis=-1, keepdims=True) * inv_d
    eps = float(np.asarray(1e-5, dtype=BF16))
    std = _rb(jnp.sqrt(_rb(_rb(var) + eps)))
    return _rb(_rb(x - _rb(mean)) * (1.0 / std))


def make_plan(c, pre):
    nv = c["nv"]
    attn = 80 - 16 * nv
    cost = dict(F=128 if pre else 160, Q=32 if pre else 40, K=32 if pre else 40, V=40, S=attn, P=attn, O=80)
    seq = [("F", 0)]
    vlag = c["vlag"]
    done = set()
    def add(k, a):
        if (k, a) not in done:
            done.add((k, a)); seq.append((k, a))
    for t in range(2, 32 + vlag):
        if t < 32: add("Q", t)
        for x in range(0, t - vlag + 1): add("V", x)
        if t < 32: add("K", t)
        for g in range(4):
            if t == 8 * g + 7 + c["slag"][g]: add("S", g)
            if t == 8 * g + 7 + c["plag"]: add("P", g)
            for n in range(4):
                if t == 8 * g + 7 + c["olag"] + n * c["ostep"]: add("O", 4 * g + n)
    for tok in c["tail"].split():
        if tok[0] == "O":
            for n in range(4): add("O", 4 * int(tok[1]) + n)
        else: add(tok[0], int(tok[1]))
    start, now = {}, 0
    for item in seq:
        start[item] = now; now += cost[item[0]]
    ev = []
    def bgtask(task, emit, tie):
        ev.append((emit, len(ev), task))
        if tie is not None: ev.append((tie, len(ev), ("tie", task)))
    bgtask(("side", 0), now - c["e_fin"], now - c["t_fin"])
    bgtask(("side", 1), now - c["e_nxt"], now - c["t_nxt"] if c["t_nxt"] else None)
    for g in range(4):
        s0 = start["S", g] + attn; p0 = start["P", g]
        for j in range(4):
            emit = s0 + 1 + j * max(0, p0 - s0 - c["softlat"]) // 4
            tie = emit + c["softlat"]
            bgtask(("soft", 4 * g + j), emit, tie if tie < p0 and c["stie"] else None)
    if nv:
        for hd in range(32):
            t1 = c["w0"] + (c["wend"] - c["w0"]) * hd // 31
            rdy = start.get(("K", hd), 0) + 41
            t1 = max(t1, rdy, 1)
            t2 = max(t1 + c["wgap"], start["V", hd] + 41)
            dead = start["O", 4 * (hd // 8)]
            t2 = min(t2, dead); t1 = min(t1, t2)
            bgtask(("w1", hd), t1, t1 + c["w1lat"] if c["w1lat"] and t1 + c["w1lat"] < dead else None)
            bgtask(("w2", hd), t2, t2 + c["w2lat"] if t2 + c["w2lat"] < dead else None)
    ev.sort()
    plan = []
    for item in seq:
        while ev and ev[0][0] <= start[item]:
            plan.append(ev.pop(0)[2])
        plan.append(item)
    return plan


def _kernel(x_hbm, mem0_hbm, wq_hbm, wk_hbm, wv_hbm, wo_hbm, wr_hbm, wg_hbm, wu_hbm, wd_hbm,
            out_hbm,
            raw, wq, wk, wv, wo, wg, wu, wd, mem0, wr, xres, x1buf, xtail, ntail, qpre, kpre, hbuf, obuf, fixbuf, kbuf, vbuf, zbuf, wcap, scap,
            sems):
    n_seg, seg, d_model = x_hbm.shape
    n_mem = mem0.shape[0]
    n_heads, _, dh = wq.shape
    rows = n_mem + seg
    n_pairs = n_heads // 2
    n_groups = n_pairs // PAIRS_PER_GROUP
    n_col = d_model // LANES
    scale = dh ** -0.5
    head = seg - SUB
    xch = CFG["xch"]
    first = 16
    PU = CFG["pu"]

    sem_ids = iter(range(3 * n_pairs, sems.shape[0]))

    def copy(src, dst):
        return pltpu.make_async_copy(src, dst, sems.at[next(sem_ids)])

    per = n_seg // xch
    tail_copies = [copy(x_hbm.at[pl.ds(j * per, per), pl.ds(head, SUB), :], xtail.at[pl.ds(j * per, per)])
                   for j in range(xch)]

    def pair_copy(i, p):
        src = (wq_hbm, wk_hbm, wv_hbm)[i].bitcast(U32)
        return pltpu.make_async_copy(src.at[:, p, :], raw.at[i * n_pairs + p], sems.at[i * n_pairs + p])

    early = [copy(mem0_hbm, mem0), copy(wr_hbm, wr), copy(x_hbm.at[pl.ds(0, first)], xres.at[pl.ds(1, first)])]
    early += [copy(wo_hbm.bitcast(U32).at[:, pl.ds(n * LANES, LANES)], wo.at[n]) for n in range(n_col)]
    x_rest = copy(x_hbm.at[pl.ds(first, n_seg - first)], xres.at[pl.ds(1 + first, n_seg - first)])
    mlp_copies = [copy(src.bitcast(U32), dst) for src, dst in ((wg_hbm, wg), (wu_hbm, wu), (wd_hbm, wd))]
    out_sem = sems.at[next(sem_ids)]
    for c in tail_copies:
        c.start()
    for p in range(n_pairs):
        pair_copy(0, p).start()
    for p in range(n_pairs):
        pair_copy(1, p).start()
        pair_copy(2, p).start()
    for c in early + ([] if CFG["stop"] else [x_rest] + mlp_copies):
        c.start()

    zeros = jnp.zeros((seg, d_model), BF16)
    xres[0] = zeros
    xres[n_seg + 1] = zeros
    obuf[...] = jnp.zeros(obuf.shape, F32)

    for j in range(xch):
        tail_copies[j].wait()
        t = xtail[pl.ds(j * per, per)].astype(F32).reshape(per * SUB, d_model)
        ntail[pl.ds(j * per * SUB // 2, per * SUB // 2), :] = pltpu.bitcast(_layernorm(t).astype(BF16), U32)

    def split(i, p):
        even = raw[i * n_pairs + p, pl.ds(0, d_model // 2, stride=2), :]
        odd = raw[i * n_pairs + p, pl.ds(1, d_model // 2, stride=2), :]
        halves = ((even & np.uint32(0xFFFF)) | (odd << 16), (even >> 16) | (odd & np.uint32(0xFFFF0000)))
        for j, half in enumerate(halves):
            (wq, wk, wv)[i][2 * p + j] = half
            if i < 2:
                (qpre, kpre)[i][2 * p + j] = _mm(_w(ntail[...]), _w(half))

    def load_pairs(which, lo, hi, unroll):
        def body(it, carry):
            ps = [lo + it * unroll + u for u in range(unroll)]
            for p in ps:
                for i in which:
                    pair_copy(i, p).wait()
            for p in ps:
                for i in which:
                    split(i, p)
            return carry
        if hi - lo == unroll:
            body(0, 0)
        else:
            lax.fori_loop(0, (hi - lo) // unroll, body, 0)

    for lo, hi, unroll in ([[0, 16, 1]] if CFG["only"] >= 0 else CFG["qplan"]):
        load_pairs((0,), lo, hi, unroll)
    load_pairs((1, 2), 0, n_pairs, 1 if CFG['only'] >= 0 else PU)
    for c in early:
        c.wait()
    if CFG["stop"]:
        return

    NV = CFG["nv"] * SUB
    qrows = rows - NV
    r = lax.broadcasted_iota(jnp.int32, (2 * qrows, 2 * rows), 0)
    c = lax.broadcasted_iota(jnp.int32, (2 * qrows, 2 * rows), 1)
    r_hi, c_hi = r >= qrows, c >= rows
    ri = jnp.where(r_hi, r - qrows, r)
    ci = jnp.where(c_hi, c - rows, c)
    same_head = r_hi == c_hi
    visible = same_head & ((ri < n_mem) | (ri + NV >= ci))
    fill = jnp.where(same_head, -1e9 / scale, -np.inf).astype(F32)
    exp2_scale = float(scale * np.log2(np.e))
    w_r = wr[...].astype(F32).reshape(1, d_model)
    sub = lax.broadcasted_iota(jnp.int32, (SUB, 1), 0)

    kbuf[:SUB, :] = jnp.zeros((SUB, dh), F32)
    vbuf[:SUB, :] = jnp.zeros((SUB, dh), F32)
    for j in range(SUB):
        wcap[j] = jnp.where(lax.broadcasted_iota(jnp.int32, (SUB, LANES), 0) >= j, np.inf, -np.inf).astype(F32)
    zbuf[...] = jnp.zeros(zbuf.shape, F32)
    scap[...] = jnp.where(visible, np.inf, fill)

    def tree(fn, xs):
        while len(xs) > 1:
            xs = [fn(xs[i], xs[i + 1]) if i + 1 < len(xs) else xs[i] for i in range(0, len(xs), 2)]
        return xs[0]

    def cat(parts, axis=0):
        return jnp.concatenate(parts, axis=axis)

    def attention(mem, tok, pre_rows, side, cfg):
        q, k, v, sc, e, inv, o = {}, {}, {}, {}, {}, {}, {}
        qs, ks, vs, ss, ov, ties = {}, {}, {}, {}, {}, []
        acc = [None] * n_col
        h = cat([tok, mem])
        qp, kp = (None, None) if pre_rows is None else (qpre, kpre)

        def tied(lhs):
            if not ties:
                return lhs
            val = tree(jnp.minimum, ties)
            ties.clear()
            first = lhs[:SUB, :LANES]
            first = jnp.maximum(first, jnp.minimum(first, val))
            return cat([cat([first, lhs[:SUB, LANES:]], 1), lhs[SUB:]])

        def pairs(g):
            return range(g * PAIRS_PER_GROUP, (g + 1) * PAIRS_PER_GROUP)

        def lhs_for(pre):
            return h if pre is None else cat([h[:head], h[seg:]])

        def arrange(t, pre, hd):
            if pre is None:
                return cat([t[seg:], t[:seg]])
            return cat([t[head:], t[:head], pre[hd, pre_rows, :]])

        def project(w, pre, hd):
            return arrange(_mm(tied(lhs_for(pre)), _w(w[hd])), pre, hd)

        def keep(buf, hd, t):
            if NV and CFG['bc'] == 'mem':
                buf[pl.ds(SUB + hd * (n_mem + NV), n_mem + NV), :] = t[:n_mem + NV]

        def put_q(hd, t):
            qs[hd] = t
            if hd % 2:
                q[hd // 2] = cat([qs[j][a:b] for j in (hd - 1, hd) for a, b in ((0, n_mem), (n_mem + NV, rows))])

        def put_k(hd, t):
            ks[hd] = t
            keep(kbuf, hd, t)
            if hd % 2:
                k[hd // 2] = cat([ks[hd - 1], t]).astype(BF16)

        def put_v(hd, t):
            vs[hd] = t
            keep(vbuf, hd, t)
            if hd % 2:
                v[hd // 2] = cat([vs[hd - 1], t]).astype(BF16)

        def first_pair(_):
            cut = CFG["ksplit"] * LANES
            lhs = lhs_for(qp)
            ws = [wq.at[0], wq.at[1], wk.at[0], wk.at[1]]
            lo = cat([_w(w[:cut // 2, :]) for w in ws], 1)
            hi = cat([_w(w[cut // 2:, :]) for w in ws], 1)
            t = _mm(lhs[:, :cut], lo)
            t = _mm(lhs[:, cut:], hi) + t
            for j in range(2):
                put_q(j, arrange(t[:, j * dh:(j + 1) * dh], qp, j))
                put_k(j, arrange(t[:, (2 + j) * dh:(3 + j) * dh], kp, j))

        def S(g):
            for p in pairs(g):
                sc[p] = _mm_nt(q[p], k[p])

        def soft(p):
            s = jnp.minimum(sc[p], scap[...])
            e[p] = jnp.exp2((s - jnp.max(s, axis=1, keepdims=True)) * exp2_scale)
            inv[p] = pltpu.reciprocal(jnp.sum(e[p], axis=1, keepdims=True), approx=True)
            return tree(jnp.minimum, [inv[p][a:a + SUB] for a in range(0, 2 * qrows, SUB)])

        def P(g):
            for p in pairs(g):
                o[p] = _mm(e[p], v[p]) * inv[p]

        def O(gn):
            g, n = divmod(gn, n_col)
            lhs = cat([cat([o[p][j * qrows:j * qrows + n_mem], *([ov[2 * p + j]] if NV else []),
                            o[p][j * qrows + n_mem:(j + 1) * qrows]]) for p in pairs(g) for j in range(2)], 1)
            width = lhs.shape[1] // 2
            t = _mm(tied(lhs), _w(wo[n, pl.ds(g * width, width), :]))
            acc[n] = (zero_acc[n] if acc[n] is None else acc[n]) + t

        def turns(t):
            return [t] + [pltpu.roll(t, r, 0) for r in range(1, SUB)]

        def block(buf, vals, hd, j):
            if CFG["bc"] == "mem":
                return buf[pl.ds(SUB + hd * (n_mem + NV) + j * SUB, SUB), :]
            return vals[hd][j * SUB:(j + 1) * SUB]

        def w1(hd):
            nb = NV // SUB
            qb = [qs[hd][n_mem + b * SUB:n_mem + (b + 1) * SUB] * exp2_scale for b in range(nb)]
            out = [[] for _ in range(nb)]
            for j in range(nb + 1):
                for r, kr in enumerate(turns(block(kbuf, ks, hd, j))):
                    for b in range(max(j - 1, 0), nb):
                        sj = jnp.sum(qb[b] * kr, axis=1, keepdims=True)
                        out[b].append(jnp.minimum(sj, wcap[r]) if j == b + 1 and r else sj)
            ss[hd] = [(x, functools.reduce(jnp.maximum, x)) for x in out]
            return ss[hd][-1][1]

        def w2(hd):
            nb = NV // SUB
            l, a = [None] * nb, [None] * nb
            for j in range(nb + 1):
                for r, vr in enumerate(turns(block(vbuf, vs, hd, j))):
                    for b in range(max(j - 1, 0), nb):
                        ej = jnp.exp2(ss[hd][b][0][j * SUB + r] - ss[hd][b][1])
                        t = ej * vr
                        l[b], a[b] = (ej, t) if l[b] is None else (l[b] + ej, a[b] + t)
            outs = [a[b] * pltpu.reciprocal(l[b], approx=True) for b in range(nb)]
            ov[hd] = cat(outs)
            return tree(jnp.minimum, outs)

        zero_acc = [zbuf[...] for _ in range(n_col)]
        mxu = dict(F=first_pair, S=S, P=P, O=O,
                   Q=lambda hd: put_q(hd, project(wq, qp, hd)),
                   K=lambda hd: put_k(hd, project(wk, kp, hd)),
                   V=lambda hd: put_v(hd, project(wv, None, hd)))
        bg = dict(w1=w1, w2=w2, soft=soft, side=lambda i: side[i]())
        pending = {}
        for kind, a in make_plan(cfg, pre_rows is not None):
            if kind in mxu:
                mxu[kind](a)
            elif kind == "tie":
                ties.append(pending.pop(a))
            else:
                pending[kind, a] = bg[kind](a)
        return cat(acc, 1)

    def finish_rows(i, o_tok, best, best_row):
        x1 = _rb(xres[i].astype(F32) + _rb(o_tok))
        x1buf[i] = x1.astype(BF16)
        n1 = _layernorm(x1)
        xres[i] = (x1 + n1).astype(BF16)
        score = _rb(jnp.sum(n1 * w_r, axis=-1, keepdims=True))
        score = jnp.where(i > 0, score, -np.inf)
        for j in range(seg // SUB):
            sj = score[SUB * j:SUB * (j + 1)]
            better = sj > best
            best = jnp.where(better, sj, best)
            best_row = jnp.where(better, (i - 1) * seg + SUB * j + sub, best_row)
        return best, best_row

    def attention_layer(first_layer):
        U = CFG["u0"] if first_layer else CFG["u1"]
        order = dict(CFG, **(CFG["p0"] if first_layer else CFG["p1"]))

        def step(it, carry):
            mem, best, best_row = carry
            if first_layer:
                @pl.when(it == 1)
                def _():
                    x_rest.wait()
            else:
                @pl.when(it > 1)
                def _():
                    lo = (it - 2) * U
                    pltpu.make_async_copy(xres.at[pl.ds(lo + 1, U)], out_hbm.at[pl.ds(lo, U)], out_sem).start()
            st = dict(best=best, best_row=best_row, tok=hbuf[...], o=obuf[...])
            for u in range(U):
                s = it * U + u
                def fin(s=s):
                    st["best"], st["best_row"] = finish_rows(s, st["o"], st["best"], st["best_row"])
                    return st["best"]
                def nxt(s=s):
                    st["nxt"] = _layernorm(xres[s + 2].astype(F32))
                    return tree(jnp.minimum, [st["nxt"][a:a + SUB, -LANES:] for a in range(0, seg, SUB)])
                pre_rows = pl.ds(pl.multiple_of(s * SUB, SUB), SUB) if first_layer else None
                out = attention(mem, st["tok"], pre_rows, (fin, nxt), order)
                mem = out[:n_mem]
                st["tok"] = st["nxt"]; st["o"] = out[n_mem:]
            hbuf[...] = st["tok"]
            obuf[...] = st["o"]
            return mem, st["best"], st["best_row"]

        hbuf[...] = _layernorm(xres[1].astype(F32))
        init = (mem0[...].astype(F32),
                jnp.full((SUB, 1), -np.inf, F32),
                jnp.zeros((SUB, 1), jnp.int32))
        _, best, best_row = lax.fori_loop(0, (CFG["n0"] if first_layer else CFG["n1"]) // U, step, init)
        return finish_rows(n_seg, obuf[...], best, best_row)

    BR = CFG["brows"]

    def routed_update(best, best_row):
        top = jnp.max(best, axis=0, keepdims=True)
        row = jnp.min(jnp.where(best == top, best_row, n_seg * seg - 1).astype(F32))
        row = jnp.clip(row.astype(jnp.int32), 0, n_seg * seg - 1)
        s = row // seg
        blk = pl.ds(pl.multiple_of(row % seg // BR * BR, BR), BR)
        x1 = x1buf[s + 1, blk, :].astype(F32)
        n1 = _layernorm(x1)
        score = _rb(jnp.sum(n1 * w_r, axis=-1, keepdims=True))
        gate = _rb(_mm(n1, _w(wg[...])))
        gate = _rb(gate * _rb(jax.nn.sigmoid(gate)))
        up = _rb(_mm(n1, _w(wu[...])))
        y = _rb(_mm(_rb(gate * up), _w(wd[...])))
        y = _rb(y * _rb(jax.nn.sigmoid(score)))
        chosen = lax.broadcasted_iota(jnp.int32, (BR, 1), 0) == row % BR
        return s, blk, (x1 + _rb(n1 + jnp.where(chosen, y, 0.0))).astype(BF16)

    if CFG["only"] >= 0:
        best, best_row = attention_layer(CFG["only"] == 0)
        fixbuf[...] = jnp.broadcast_to(best + best_row.astype(F32), fixbuf.shape).astype(BF16)
        pltpu.sync_copy(fixbuf, out_hbm.at[0, pl.ds(0, BR), :])
        pltpu.sync_copy(x1buf.at[pl.ds(1, n_seg)], out_hbm)
        pltpu.sync_copy(xres.at[pl.ds(1, n_seg)], out_hbm)
        return
    best, best_row = attention_layer(True)
    for cp in mlp_copies:
        cp.wait()
    s, blk, new = routed_update(best, best_row)
    xres[s + 1, blk, :] = new

    best, best_row = attention_layer(False)
    lo = CFG["n1"] - 2 * CFG["u1"]
    pltpu.make_async_copy(xres.at[pl.ds(lo + 1, n_seg - lo)], out_hbm.at[pl.ds(lo, n_seg - lo)], out_sem).start()
    s, blk, new = routed_update(best, best_row)
    fixbuf[...] = new
    pltpu.make_async_copy(xres.at[pl.ds(1, n_seg)], out_hbm, out_sem).wait()
    fix = pltpu.make_async_copy(fixbuf, out_hbm.at[s, blk, :], out_sem)
    fix.start()
    fix.wait()


def pallas_interleave_layers__memory_aug_recurrent_mem_tr__moe_arch_mod__prompt_kernel(
    A_x, A_mem0, A_Wq, A_Wk, A_Wv, A_Wo, A_seg_len, B_x, B_w_r, B_w_gate, B_w_up, B_w_down,
):
    del B_x
    batch, seq, d_model = A_x.shape
    assert batch == 1
    n_heads, dh = A_Wq.shape[1:]
    n_mem = A_mem0.shape[1]
    seg = int(A_seg_len)
    n_seg = seq // seg
    d_ff = B_w_gate.shape[1]

    any_spec = pl.BlockSpec(memory_space=pl.ANY)
    out = pl.pallas_call(
        _kernel,
        out_shape=jax.ShapeDtypeStruct((n_seg, seg, d_model), A_x.dtype),
        in_specs=[any_spec] * 10,
        out_specs=any_spec,
        scratch_shapes=[
            pltpu.VMEM((3 * n_heads // 2, d_model, dh), U32),
            pltpu.VMEM((n_heads, d_model // 2, dh), U32),
            pltpu.VMEM((n_heads, d_model // 2, dh), U32),
            pltpu.VMEM((n_heads, d_model // 2, dh), U32),
            pltpu.VMEM((d_model // LANES, n_heads * dh // 2, LANES), U32),
            pltpu.VMEM((d_model // 2, d_ff), U32),
            pltpu.VMEM((d_model // 2, d_ff), U32),
            pltpu.VMEM((d_ff // 2, d_model), U32),
            pltpu.VMEM((n_mem, d_model), BF16),
            pltpu.VMEM((d_model,), BF16),
            pltpu.VMEM((n_seg + 2, seg, d_model), BF16),
            pltpu.VMEM((n_seg + 1, seg, d_model), BF16),
            pltpu.VMEM((n_seg, SUB, d_model), BF16),
            pltpu.VMEM((n_seg * SUB // 2, d_model), U32),
            pltpu.VMEM((n_heads, n_seg * SUB, dh), F32),
            pltpu.VMEM((n_heads, n_seg * SUB, dh), F32),
            pltpu.VMEM((seg, d_model), F32),
            pltpu.VMEM((seg, d_model), F32),
            pltpu.VMEM((CFG["brows"], d_model), BF16),
            pltpu.VMEM((SUB + n_heads * (n_mem + CFG["nv"] * SUB), dh), F32),
            pltpu.VMEM((SUB + n_heads * (n_mem + CFG["nv"] * SUB), dh), F32),
            pltpu.VMEM((n_mem + seg, LANES), F32),
            pltpu.VMEM((SUB, SUB, LANES), F32),
            pltpu.VMEM((2 * (n_mem + seg - CFG["nv"] * SUB), 2 * (n_mem + seg)), F32),
            pltpu.SemaphoreType.DMA((3 * n_heads // 2 + CFG["xch"] + 8 + d_model // LANES,)),
        ],
        compiler_params=pltpu.CompilerParams(vmem_limit_bytes=100 * 1024 * 1024, flags=CFG["flags"] or None,
            disable_bounds_checks=bool(CFG["nochk"]), disable_semaphore_checks=bool(CFG["nochk"])),
    )(
        A_x.reshape(n_seg, seg, d_model),
        A_mem0.reshape(n_mem, d_model),
        A_Wq,
        A_Wk,
        A_Wv,
        A_Wo.reshape(n_heads * dh, d_model),
        B_w_r,
        B_w_gate,
        B_w_up,
        B_w_down,
    )
    return out.reshape(batch, seq, d_model)
```

```python
import functools

import jax
import jax.numpy as jnp
import numpy as np
from jax import lax
import jax.experimental.pallas as pl
import jax.experimental.pallas.tpu as pltpu

F32 = jnp.float32
BF16 = jnp.bfloat16
U32 = jnp.uint32
LANES = 128
SUB = 8
N_LAYERS = 2
GROUP = 8
UNROLL = 8
TAIL_COPIES = 2

PLAN = dict(
    v_lag=2, score_lag=3, mix_lag=11, out_lag=18,
    lead_first=400, lead_last=4000, lead_score_due=450, lead_mix_due=350,
    finish_at=900, finish_due=100, norm_at=1150,
)


def _mm(a, b):
    return lax.dot_general(a, b, (((1,), (0,)), ((), ())), preferred_element_type=F32)


def _mm_nt(a, b):
    return lax.dot_general(a, b, (((1,), (1,)), ((), ())), preferred_element_type=F32)


def _cat(parts, axis=0):
    return jnp.concatenate(parts, axis=axis)


def _rb(x):
    return x.astype(BF16).astype(F32)


def _bf16(words):
    return pltpu.bitcast(words, BF16)


def _after(x, other):
    return jnp.maximum(x, jnp.minimum(x, other))


def _layernorm(x):
    inv_d = 1.0 / x.shape[-1]
    mean = jnp.sum(x, axis=-1, keepdims=True) * inv_d
    cen = x - mean
    var = jnp.sum(cen * cen, axis=-1, keepdims=True) * inv_d
    eps = float(np.asarray(1e-5, dtype=BF16))
    std = _rb(jnp.sqrt(_rb(_rb(var) + eps)))
    return _rb(x - _rb(mean)) * (1.0 / std)


def _step_plan(n_heads, n_col, rows):
    n_groups = n_heads // GROUP
    mxu = [("qk_first", 0)]
    for t in range(2, n_heads + PLAN["v_lag"]):
        if t < n_heads:
            mxu.append(("q", t))
        if t >= PLAN["v_lag"]:
            mxu.append(("v", t - PLAN["v_lag"]))
        if t < n_heads:
            mxu.append(("k", t))
        for g in range(n_groups):
            since = t - (GROUP * (g + 1) - 1)
            if since == PLAN["score_lag"]:
                mxu.append(("scores", g))
            if since == PLAN["mix_lag"]:
                mxu.append(("mix", g))
            if 0 <= since - PLAN["out_lag"] < n_col:
                mxu.append(("out", (g, since - PLAN["out_lag"])))
    rest = [("scores", g) for g in range(n_groups)] + [("mix", g) for g in range(n_groups - 1)]
    rest += [("out", (g, n)) for g in range(n_groups - 2) for n in range(n_col)]
    rest += [("mix", n_groups - 1)]
    rest += [("out", (g, n)) for g in range(n_groups - 2, n_groups) for n in range(n_col)]
    mxu += [task for task in rest if task not in mxu]

    short = rows - SUB
    cycles = dict(qk_first=4 * short, q=short, k=short, v=rows, scores=2 * short, mix=2 * short,
                  out=GROUP * rows // 4)
    start, end = {}, 0
    for task in mxu:
        start[task] = end
        end += cycles[task[0]]

    vector = [
        (end - PLAN["finish_at"], ("finish", 0)),
        (end - PLAN["finish_due"], ("due", ("finish", 0))),
        (end - PLAN["norm_at"], ("norm", 0)),
    ]
    vector += [(start["scores", g] + 1, ("softmax", g)) for g in range(n_groups)]
    for hd in range(n_heads):
        needed = start["out", (hd // GROUP, 0)]
        at = PLAN["lead_first"] + (PLAN["lead_last"] - PLAN["lead_first"]) * hd // (n_heads - 1)
        at_score = max(at, start.get(("k", hd), 0) + rows + 1)
        at_mix = min(max(at_score, start["v", hd] + rows + 1), needed)
        for kind, when in (("lead_score", min(at_score, at_mix)), ("lead_mix", at_mix)):
            vector.append((when, (kind, hd)))
            if when + PLAN[kind + "_due"] < needed:
                vector.append((when + PLAN[kind + "_due"], ("due", (kind, hd))))
    vector.sort(key=lambda event: event[0])

    plan = []
    for task in mxu:
        while vector and vector[0][0] <= start[task]:
            plan.append(vector.pop(0)[1])
        plan.append(task)
    assert not vector
    return plan


def _kernel(x_hbm, mem0_hbm, wq_hbm, wk_hbm, wv_hbm, wo_hbm, wr_hbm, wg_hbm, wu_hbm, wd_hbm,
            out_hbm,
            raw, wq, wk, wv, wo, wg, wu, wd, mem0, wr, xres, xmid, xtail, ntail, qtail, ktail,
            hbuf, obuf, fixbuf, zeros, lead_cap, pair_cap, sems):
    n_seg, seg, d_model = x_hbm.shape
    n_mem = mem0.shape[0]
    n_heads, _, dh = wq.shape
    rows = n_mem + seg
    front = seg - SUB
    n_pairs = n_heads // 2
    n_col = d_model // LANES
    scale = dh ** -0.5
    exp2_scale = float(scale * np.log2(np.e))


    free_sems = iter(range(3 * n_pairs, sems.shape[0]))

    def copy(src, dst):
        return pltpu.make_async_copy(src, dst, sems.at[next(free_sems)])

    def pair_copy(i, p):
        src = (wq_hbm, wk_hbm, wv_hbm)[i].bitcast(U32)
        return pltpu.make_async_copy(src.at[:, p, :], raw.at[i * n_pairs + p], sems.at[i * n_pairs + p])

    chunk = n_seg // TAIL_COPIES
    tail_copies = [copy(x_hbm.at[pl.ds(j * chunk, chunk), pl.ds(front, SUB), :], xtail.at[pl.ds(j * chunk, chunk)])
                   for j in range(TAIL_COPIES)]
    n_first = UNROLL + 1
    x_first = copy(x_hbm.at[pl.ds(0, n_first)], xres.at[pl.ds(1, n_first)])
    step_copies = [copy(mem0_hbm, mem0), copy(wr_hbm, wr.at[pl.ds(0, d_model)])]
    step_copies += [copy(wo_hbm.bitcast(U32).at[:, pl.ds(n * LANES, LANES)], wo.at[n]) for n in range(n_col)]
    x_rest = copy(x_hbm.at[pl.ds(n_first, n_seg - n_first)], xres.at[pl.ds(1 + n_first, n_seg - n_first)])
    mlp_copies = [copy(src.bitcast(U32), dst) for src, dst in ((wg_hbm, wg), (wu_hbm, wu), (wd_hbm, wd))]
    out_sem = sems.at[next(free_sems)]

    for cp in tail_copies:
        cp.start()
    for p in range(n_pairs):
        pair_copy(0, p).start()
    x_first.start()
    for p in range(n_pairs):
        pair_copy(1, p).start()
        pair_copy(2, p).start()
    for cp in step_copies + [x_rest] + mlp_copies:
        cp.start()

    xres[0] = jnp.zeros((seg, d_model), BF16)
    xres[n_seg + 1] = jnp.zeros((seg, d_model), BF16)
    ntail[pl.ds((n_seg + 1) * SUB, SUB), :] = jnp.zeros((SUB, d_model), F32)
    obuf[...] = jnp.zeros(obuf.shape, F32)
    zeros[...] = jnp.zeros(zeros.shape, F32)
    for j in range(SUB):
        seen = lax.broadcasted_iota(jnp.int32, (SUB, LANES), 0) >= j
        lead_cap[j] = jnp.where(seen, np.inf, -1e9 * np.log2(np.e)).astype(F32)
    r = lax.broadcasted_iota(jnp.int32, pair_cap.shape, 0)
    c = lax.broadcasted_iota(jnp.int32, pair_cap.shape, 1)
    r_pos = jnp.where(r >= rows, r - rows, r)
    c_pos = jnp.where(c >= rows, c - rows, c)
    same_head = ((r >= rows) == (c >= rows)) & (c < 2 * rows)
    causal = jnp.where((r_pos < n_mem) | (r_pos >= c_pos), np.inf, -1e9 / scale)
    pair_cap[...] = jnp.where(same_head, causal, -np.inf).astype(F32)
    sub = lax.broadcasted_iota(jnp.int32, (SUB, 1), 0)

    def tail_rows(slot):
        return pl.ds(pl.multiple_of(slot * SUB, SUB), SUB)

    def project_tail(dst, hd, words):
        t = _mm(ntail[pl.ds(SUB, n_seg * SUB), :], _bf16(words))
        dst[hd] = t
        return t

    def normed_tokens(slot):
        return _cat([_layernorm(xres[slot].astype(F32)[:front]), ntail[tail_rows(slot), :]])

    def norm_tail(j):
        t = xtail[pl.ds(j * chunk, chunk)].astype(F32).reshape(chunk * SUB, d_model)
        ntail[pl.ds((1 + j * chunk) * SUB, chunk * SUB), :] = _layernorm(t)

    def split_pair(i, p):
        even = raw[i * n_pairs + p, pl.ds(0, d_model // 2, stride=2), :]
        odd = raw[i * n_pairs + p, pl.ds(1, d_model // 2, stride=2), :]
        return (even & np.uint32(0xFFFF)) | (odd << 16), (even >> 16) | (odd & np.uint32(0xFFFF0000))

    def load_q(p):
        for j, words in enumerate(split_pair(0, p)):
            wq[2 * p + j] = words
            project_tail(qtail, 2 * p + j, words)

    for j in range(TAIL_COPIES - 1):
        tail_copies[j].wait()
        norm_tail(j)
    tail_copies[-1].wait()
    pair_copy(0, 0).wait()
    norm_tail(TAIL_COPIES - 1)
    load_q(0)

    @pl.loop(1, n_pairs, step=3)
    def _(first):
        for u in range(3):
            pair_copy(0, first + u).wait()
        for u in range(3):
            load_q(first + u)

    x_first.wait()

    @pl.loop(0, n_pairs, step=n_pairs // 2)
    def _(first):
        batch = [first + u for u in range(n_pairs // 2)]
        for p in batch:
            pair_copy(1, p).wait()
            pair_copy(2, p).wait()
        hbuf[...] = normed_tokens(1)
        for p in batch:
            projected = []
            for j, words in enumerate(split_pair(1, p)):
                wk[2 * p + j] = words
                projected.append(project_tail(ktail, 2 * p + j, words)[SUB:SUB + words.shape[0]])
            for j, words in enumerate(split_pair(2, p)):
                paced = _after(pltpu.bitcast(words, jnp.int32), pltpu.bitcast(projected[j], jnp.int32))
                wv[2 * p + j] = pltpu.bitcast(paced, U32)

    for cp in step_copies:
        cp.wait()
    w_r = wr[pl.ds(0, d_model)].astype(F32).reshape(1, d_model)

    def attend(s, mem, tok, row_tasks):
        q, k, v, k_pair, v_pair, score, expo, inv, mixed, lead = ({} for _ in range(10))
        due, latest = [], []
        acc = [zeros[:rows, :] for _ in range(n_col)]
        h_all = _cat([tok, mem])
        h_front = _cat([tok[:front], mem])
        on_mxu = ((0, n_mem), (n_mem + SUB, rows))

        def matmul(lhs, words):
            if due:
                corner = _after(lhs[:SUB, :LANES], functools.reduce(jnp.minimum, due))
                lhs = _cat([_cat([corner, lhs[:SUB, LANES:]], 1), lhs[SUB:]])
                due.clear()
            return _mm(lhs, _bf16(words))

        def with_tail(t, tail, hd):
            return _cat([t[front:], t[:front], tail[hd, tail_rows(s), :]])

        def pairs(g):
            return range(g * GROUP // 2, (g + 1) * GROUP // 2)

        def pack_pair(dst, src, hd):
            if hd % 2:
                dst[hd // 2] = _cat([src[hd - 1], src[hd]]).astype(BF16)

        def qk_first(_):
            cut = d_model - LANES
            ws = [wq.at[0], wq.at[1], wk.at[0], wk.at[1]]
            t = _mm(h_front[:, :cut], _cat([_bf16(w[:cut // 2, :]) for w in ws], 1))
            t = _mm(h_front[:, cut:], _cat([_bf16(w[cut // 2:, :]) for w in ws], 1)) + t
            for hd in range(2):
                q[hd] = with_tail(t[:, hd * dh:(hd + 1) * dh], qtail, hd)
                k[hd] = with_tail(t[:, (2 + hd) * dh:(3 + hd) * dh], ktail, hd)
            pack_pair(k_pair, k, 1)

        def project_q(hd):
            t = matmul(h_front, wq[hd])
            latest.append(t[:SUB])
            q[hd] = with_tail(t, qtail, hd)

        def project_k(hd):
            t = matmul(h_front, wk[hd])
            latest.append(t[:SUB])
            k[hd] = with_tail(t, ktail, hd)
            pack_pair(k_pair, k, hd)

        def project_v(hd):
            t = matmul(h_all, wv[hd])
            latest.append(t[:SUB])
            v[hd] = _cat([t[seg:], t[:seg]])
            pack_pair(v_pair, v, hd)

        def scores(g):
            for p in pairs(g):
                q_pair = _cat([q[2 * p + j][a:b] for j in range(2) for a, b in on_mxu])
                score[p] = _mm_nt(q_pair, k_pair[p])

        def softmax(g):
            for p in pairs(g):
                cap = _cat([pair_cap[j * rows + a:j * rows + b, :] for j in range(2) for a, b in on_mxu])
                t = _cat([score[p], jnp.zeros((cap.shape[0], LANES - 2 * rows), F32)], 1)
                t = jnp.minimum(t, cap)
                t = jnp.exp2((t - jnp.max(t, axis=1, keepdims=True)) * exp2_scale)
                inv[p] = pltpu.reciprocal(jnp.sum(t, axis=1, keepdims=True), approx=True)
                expo[p] = t[:, :2 * rows]

        def mix(g):
            for p in pairs(g):
                mixed[p] = _mm(expo[p], v_pair[p]) * inv[p]

        def rotations(t):
            for block in range(2):
                keys = t[block * SUB:(block + 1) * SUB]
                for shift in range(SUB):
                    yield block * shift, pltpu.roll(keys, shift, 0) if shift else keys

        def lead_score(hd):
            scaled = q[hd][n_mem:n_mem + SUB] * exp2_scale
            ts = []
            for first_seen, keys in rotations(k[hd]):
                t = jnp.sum(scaled * keys, axis=1, keepdims=True)
                ts.append(jnp.minimum(t, lead_cap[first_seen]) if first_seen else t)
            lead[hd] = ts, functools.reduce(jnp.maximum, ts)
            return lead[hd][1]

        def lead_mix(hd):
            ts, top = lead[hd]
            top = _after(top, latest[-2])
            total = out = None
            for t, (_, values) in zip(ts, rotations(v[hd])):
                t = jnp.exp2(t - top)
                total, out = (t, t * values) if out is None else (total + t, out + t * values)
            lead[hd] = out * pltpu.reciprocal(total, approx=True)
            return lead[hd]

        def project_out(task):
            g, n = task
            heads = []
            for hd in range(g * GROUP, (g + 1) * GROUP):
                t = mixed[hd // 2][hd % 2 * (rows - SUB):(hd % 2 + 1) * (rows - SUB)]
                heads.append(_cat([t[:n_mem], lead[hd], t[n_mem:]]))
            words = GROUP * dh // 2
            acc[n] = acc[n] + matmul(_cat(heads, 1), wo[n, pl.ds(g * words, words), :])
            latest.extend([acc[n][:SUB]] * 2)

        tasks = dict(row_tasks, qk_first=qk_first, q=project_q, k=project_k, v=project_v, scores=scores,
                     softmax=softmax, mix=mix, lead_score=lead_score, lead_mix=lead_mix, out=project_out)
        results = {}
        for kind, arg in _step_plan(n_heads, n_col, rows):
            if kind == "due":
                due.append(results[arg])
            else:
                results[kind, arg] = tasks[kind](arg)
        out = _cat(acc, 1)
        return out[:n_mem], out[n_mem:]

    def finish(slot, attn, best):
        best_score, best_row, best_norm = best
        x1 = _rb(xres[slot].astype(F32) + _rb(attn))
        xmid[slot] = x1.astype(BF16)
        n1 = _rb(_layernorm(x1))
        x2 = (x1 + n1).astype(BF16)
        xres[slot] = x2
        ntail[tail_rows(slot), :] = _layernorm(x2.astype(F32)[front:])
        score = _rb(jnp.sum(n1 * w_r, axis=-1, keepdims=True))
        score = jnp.where(slot > 0, score, -np.inf)
        for j in range(0, seg, SUB):
            better = score[j:j + SUB] > best_score
            best_score = jnp.where(better, score[j:j + SUB], best_score)
            best_row = jnp.where(better, (slot - 1) * seg + j + sub, best_row)
            best_norm = jnp.where(better, n1[j:j + SUB], best_norm)
        return best_score, best_row, best_norm

    def out_copy(first, count):
        return pltpu.make_async_copy(xres.at[pl.ds(first + 1, count)], out_hbm.at[pl.ds(first, count)], out_sem)

    @pl.loop(0, N_LAYERS)
    def _(layer):
        is_first, is_last = layer == 0, layer == N_LAYERS - 1

        def steps(it, carry):
            mem, best = carry

            @pl.when(is_first & (it == 1))
            def _():
                x_rest.wait()

            @pl.when(is_last & (it >= 2))
            def _():
                out_copy((it - 2) * UNROLL, UNROLL).start()

            live = dict(best=best, tok=hbuf[...], attn=obuf[...])
            for u in range(UNROLL):
                s = it * UNROLL + u

                def finish_previous(_, s=s):
                    live["best"] = finish(s, live["attn"], live["best"])
                    return live["best"][0]

                def norm_next(_, s=s):
                    live["tok"] = normed_tokens(s + 2)

                mem, live["attn"] = attend(s, mem, live["tok"], dict(finish=finish_previous, norm=norm_next))
            hbuf[...] = live["tok"]
            obuf[...] = live["attn"]
            return mem, live["best"]

        best = (jnp.full((SUB, 1), -np.inf, F32), jnp.zeros((SUB, 1), jnp.int32), jnp.zeros((SUB, d_model), F32))
        _, best = lax.fori_loop(0, n_seg // UNROLL, steps, (mem0[...].astype(F32), best))

        @pl.when(is_first)
        def _():
            for cp in mlp_copies:
                cp.wait()

        score, row, n1 = finish(n_seg, obuf[...], best)

        @pl.when(is_last)
        def _():
            out_copy(n_seg - 2 * UNROLL, 2 * UNROLL).start()

        gate = _rb(_mm(n1, _bf16(wg[...])))
        gate = _rb(gate * _rb(jax.nn.sigmoid(gate)))
        up = _rb(_mm(n1, _bf16(wu[...])))
        y = _rb(_mm(_rb(gate * up), _bf16(wd[...])))
        update = _rb(n1 + _rb(y * _rb(jax.nn.sigmoid(score))))

        top = jnp.max(score, axis=0, keepdims=True)
        row = jnp.min(jnp.where(score == top, row, n_seg * seg - 1).astype(F32))
        row = jnp.clip(row.astype(jnp.int32), 0, n_seg * seg - 1)
        s = row // seg
        block = pl.ds(pl.multiple_of(row % seg // SUB * SUB, SUB), SUB)
        routed = (sub == row % SUB) & (score > -np.inf)
        fixed = jnp.where(routed, xmid[s + 1, block, :].astype(F32) + update, xres[s + 1, block, :].astype(F32))
        fixed = fixed.astype(BF16)

        @pl.when(jnp.logical_not(is_last))
        def _():
            xres[s + 1, block, :] = fixed

            @pl.when(row % seg >= front)
            def _():
                ntail[tail_rows(s + 1), :] = _layernorm(fixed.astype(F32))

            @pl.loop(0, n_heads, step=GROUP)
            def _(first):
                hbuf[...] = normed_tokens(1)
                for u in range(GROUP):
                    project_tail(qtail, first + u, wq[first + u])
                    project_tail(ktail, first + u, wk[first + u])

        @pl.when(is_last)
        def _():
            fixbuf[:SUB, :] = fixed
            out_copy(0, n_seg).wait()
            fix_copy = pltpu.make_async_copy(fixbuf.at[pl.ds(0, SUB)], out_hbm.at[s, block, :], out_sem)
            fix_copy.start()
            fix_copy.wait()


def pallas_interleave_layers__memory_aug_recurrent_mem_tr__moe_arch_mod__prompt_kernel(
    A_x, A_mem0, A_Wq, A_Wk, A_Wv, A_Wo, A_seg_len, B_x, B_w_r, B_w_gate, B_w_up, B_w_down,
):
    del B_x
    batch, seq, d_model = A_x.shape
    n_heads, dh = A_Wq.shape[1:]
    n_mem = A_mem0.shape[1]
    seg = int(A_seg_len)
    n_seg = seq // seg
    d_ff = B_w_gate.shape[1]
    assert (batch, n_mem, seg, n_heads, dh) == (1, SUB, 32, 32, LANES) and n_seg % (2 * UNROLL) == 0

    any_spec = pl.BlockSpec(memory_space=pl.ANY)
    out = pl.pallas_call(
        _kernel,
        out_shape=jax.ShapeDtypeStruct((n_seg, seg, d_model), A_x.dtype),
        in_specs=[any_spec] * 10,
        out_specs=any_spec,
        scratch_shapes=[
            pltpu.VMEM((3 * n_heads // 2, d_model, dh), U32),
            pltpu.VMEM((n_heads, d_model // 2, dh), U32),
            pltpu.VMEM((n_heads, d_model // 2, dh), U32),
            pltpu.VMEM((n_heads, d_model // 2, dh), U32),
            pltpu.VMEM((d_model // LANES, n_heads * dh // 2, LANES), U32),
            pltpu.VMEM((d_model // 2, d_ff), U32),
            pltpu.VMEM((d_model // 2, d_ff), U32),
            pltpu.VMEM((d_ff // 2, d_model), U32),
            pltpu.VMEM((n_mem, d_model), BF16),
            pltpu.VMEM((SUB * d_model,), BF16),
            pltpu.VMEM((n_seg + 2, seg, d_model), BF16),
            pltpu.VMEM((n_seg + 1, seg, d_model), BF16),
            pltpu.VMEM((n_seg, SUB, d_model), BF16),
            pltpu.VMEM(((n_seg + 2) * SUB, d_model), F32),
            pltpu.VMEM((n_heads, n_seg * SUB, dh), F32),
            pltpu.VMEM((n_heads, n_seg * SUB, dh), F32),
            pltpu.VMEM((seg, d_model), F32),
            pltpu.VMEM((seg, d_model), F32),
            pltpu.VMEM((2 * SUB, d_model), BF16),
            pltpu.VMEM((64, LANES), F32),
            pltpu.VMEM((SUB, SUB, LANES), F32),
            pltpu.VMEM((96, LANES), F32),
            pltpu.SemaphoreType.DMA((3 * n_heads // 2 + TAIL_COPIES + d_model // LANES + 8,)),
        ],
        compiler_params=pltpu.CompilerParams(
            vmem_limit_bytes=100 * 1024 * 1024,
            disable_bounds_checks=True,
            disable_semaphore_checks=True,
        ),
    )(
        A_x.reshape(n_seg, seg, d_model),
        A_mem0.reshape(n_mem, d_model),
        A_Wq,
        A_Wk,
        A_Wv,
        A_Wo.reshape(n_heads * dh, d_model),
        B_w_r,
        B_w_gate,
        B_w_up,
        B_w_down,
    )
    return out.reshape(batch, seq, d_model)
```

```python
import functools

import jax
import jax.numpy as jnp
import numpy as np
from jax import lax
import jax.experimental.pallas as pl
import jax.experimental.pallas.tpu as pltpu

F32 = jnp.float32
BF16 = jnp.bfloat16
U32 = jnp.uint32
LANES = 128
SUB = 8
N_LAYERS = 2
GROUP = 8
UNROLL = 8
TAIL_COPIES = 2
Q_BATCH = 3
KV_BATCH = 8

PLAN = dict(
    v_lag=2, score_lag=3, mix_lag=11, out_lag=18,
    lead_first=400, lead_last=4000, lead_score_due=450, lead_mix_due=350,
    finish_at=900, finish_due=100, norm_at=1150,
)


def _mm(a, b):
    return lax.dot_general(a, b, (((1,), (0,)), ((), ())), preferred_element_type=F32)


def _mm_nt(a, b):
    return lax.dot_general(a, b, (((1,), (1,)), ((), ())), preferred_element_type=F32)


def _cat(parts, axis=0):
    return jnp.concatenate(parts, axis=axis)


def _rb(x):
    return x.astype(BF16).astype(F32)


def _bf16(words):
    return pltpu.bitcast(words, BF16)


def _after(x, other):
    return jnp.maximum(x, jnp.minimum(x, other))


def _layernorm(x):
    inv_d = 1.0 / x.shape[-1]
    mean = jnp.sum(x, axis=-1, keepdims=True) * inv_d
    cen = x - mean
    var = jnp.sum(cen * cen, axis=-1, keepdims=True) * inv_d
    eps = float(np.asarray(1e-5, dtype=BF16))
    std = _rb(jnp.sqrt(_rb(_rb(var) + eps)))
    return _rb(x - _rb(mean)) * (1.0 / std)


def _step_plan(n_heads, n_col, rows):
    n_groups = n_heads // GROUP
    mxu = [("qk_first", 0)]
    for t in range(2, n_heads + PLAN["v_lag"]):
        if t < n_heads:
            mxu.append(("q", t))
        if t >= PLAN["v_lag"]:
            mxu.append(("v", t - PLAN["v_lag"]))
        if t < n_heads:
            mxu.append(("k", t))
        for g in range(n_groups):
            since = t - (GROUP * (g + 1) - 1)
            if since == PLAN["score_lag"]:
                mxu.append(("scores", g))
            if since == PLAN["mix_lag"]:
                mxu.append(("mix", g))
            if 0 <= since - PLAN["out_lag"] < n_col:
                mxu.append(("out", (g, since - PLAN["out_lag"])))
    rest = [("scores", g) for g in range(n_groups)] + [("mix", g) for g in range(n_groups - 1)]
    rest += [("out", (g, n)) for g in range(n_groups - 2) for n in range(n_col)]
    rest += [("mix", n_groups - 1)]
    rest += [("out", (g, n)) for g in range(n_groups - 2, n_groups) for n in range(n_col)]
    mxu += [task for task in rest if task not in mxu]

    short = rows - SUB
    cycles = dict(qk_first=4 * short, q=short, k=short, v=rows, scores=2 * short, mix=2 * short,
                  out=GROUP * rows // 4)
    start, end = {}, 0
    for task in mxu:
        start[task] = end
        end += cycles[task[0]]

    vector = [
        (end - PLAN["finish_at"], ("finish", 0)),
        (end - PLAN["finish_due"], ("due", ("finish", 0))),
        (end - PLAN["norm_at"], ("norm", 0)),
    ]
    vector += [(start["scores", g] + 1, ("softmax", g)) for g in range(n_groups)]
    for hd in range(n_heads):
        needed = start["out", (hd // GROUP, 0)]
        at = PLAN["lead_first"] + (PLAN["lead_last"] - PLAN["lead_first"]) * hd // (n_heads - 1)
        at_score = max(at, start.get(("k", hd), 0) + rows + 1)
        at_mix = min(max(at_score, start["v", hd] + rows + 1), needed)
        for kind, when in (("lead_score", min(at_score, at_mix)), ("lead_mix", at_mix)):
            vector.append((when, (kind, hd)))
            if when + PLAN[kind + "_due"] < needed:
                vector.append((when + PLAN[kind + "_due"], ("due", (kind, hd))))
    vector.sort(key=lambda event: event[0])

    plan = []
    for task in mxu:
        while vector and vector[0][0] <= start[task]:
            plan.append(vector.pop(0)[1])
        plan.append(task)
    assert not vector
    return plan


def _kernel(x_hbm, mem0_hbm, wq_hbm, wk_hbm, wv_hbm, wo_hbm, wr_hbm, wg_hbm, wu_hbm, wd_hbm,
            out_hbm,
            raw, wq, wk, wv, wo, wg, wu, wd, mem0, wr, xres, xmid, xtail, ntail, qtail, ktail,
            hbuf, obuf, fixbuf, zeros, lead_cap, pair_cap, sems):
    n_seg, seg, d_model = x_hbm.shape
    n_mem = mem0.shape[0]
    n_heads, _, dh = wq.shape
    rows = n_mem + seg
    front = seg - SUB
    n_pairs = n_heads // 2
    n_col = d_model // LANES
    scale = dh ** -0.5
    exp2_scale = float(scale * np.log2(np.e))


    q_steps, kv_steps = (n_pairs - 1) // Q_BATCH + 1, n_pairs // KV_BATCH
    free_sems = iter(range(q_steps + kv_steps, sems.shape[0]))

    def copies(*src_dst):
        sem = sems.at[next(free_sems)]
        return [pltpu.make_async_copy(src, dst, sem) for src, dst in src_dst]

    def pair_copy(i, p):
        src = (wq_hbm, wk_hbm, wv_hbm)[i].bitcast(U32)
        sem = (p + Q_BATCH - 1) // Q_BATCH if i == 0 else q_steps + p // KV_BATCH
        return pltpu.make_async_copy(src.at[:, p, :], raw.at[i * n_pairs + p], sems.at[sem])

    chunk = n_seg // TAIL_COPIES
    tail_copies = [copies((x_hbm.at[pl.ds(j * chunk, chunk), pl.ds(front, SUB), :],
                           xtail.at[pl.ds(j * chunk, chunk)]))[0] for j in range(TAIL_COPIES)]
    n_first = UNROLL + 1
    x_first, = copies((x_hbm.at[pl.ds(0, n_first)], xres.at[pl.ds(1, n_first)]))
    step_copies = copies((mem0_hbm, mem0), (wr_hbm, wr.at[pl.ds(0, d_model)]),
                         *[(wo_hbm.bitcast(U32).at[:, pl.ds(n * LANES, LANES)], wo.at[n]) for n in range(n_col)])
    x_rest, = copies((x_hbm.at[pl.ds(n_first, n_seg - n_first)], xres.at[pl.ds(1 + n_first, n_seg - n_first)]))
    mlp_copies = copies((wg_hbm.bitcast(U32), wg), (wu_hbm.bitcast(U32), wu), (wd_hbm.bitcast(U32), wd))
    out_sem = sems.at[next(free_sems)]

    for cp in tail_copies:
        cp.start()
    for p in range(n_pairs):
        pair_copy(0, p).start()
    x_first.start()
    for p in range(n_pairs):
        pair_copy(1, p).start()
        pair_copy(2, p).start()
    for cp in step_copies + [x_rest] + mlp_copies:
        cp.start()

    xres[0] = jnp.zeros((seg, d_model), BF16)
    xres[n_seg + 1] = jnp.zeros((seg, d_model), BF16)
    ntail[pl.ds((n_seg + 1) * SUB, SUB), :] = jnp.zeros((SUB, d_model), F32)
    obuf[...] = jnp.zeros(obuf.shape, F32)
    zeros[...] = jnp.zeros(zeros.shape, F32)
    for j in range(SUB):
        seen = lax.broadcasted_iota(jnp.int32, (SUB, LANES), 0) >= j
        lead_cap[j] = jnp.where(seen, np.inf, -1e9 * np.log2(np.e)).astype(F32)
    r = lax.broadcasted_iota(jnp.int32, pair_cap.shape, 0)
    c = lax.broadcasted_iota(jnp.int32, pair_cap.shape, 1)
    r_pos = jnp.where(r >= rows, r - rows, r)
    c_pos = jnp.where(c >= rows, c - rows, c)
    same_head = ((r >= rows) == (c >= rows)) & (c < 2 * rows)
    causal = jnp.where((r_pos < n_mem) | (r_pos >= c_pos), np.inf, -1e9 / scale)
    pair_cap[...] = jnp.where(same_head, causal, -np.inf).astype(F32)
    sub = lax.broadcasted_iota(jnp.int32, (SUB, 1), 0)

    def tail_rows(slot):
        return pl.ds(pl.multiple_of(slot * SUB, SUB), SUB)

    def project_tail(dst, hd, words):
        t = _mm(ntail[pl.ds(SUB, n_seg * SUB), :], _bf16(words))
        dst[hd] = t
        return t

    def normed_tokens(slot):
        return _cat([_layernorm(xres[slot].astype(F32)[:front]), ntail[tail_rows(slot), :]])

    def norm_tail(j):
        t = xtail[pl.ds(j * chunk, chunk)].astype(F32).reshape(chunk * SUB, d_model)
        ntail[pl.ds((1 + j * chunk) * SUB, chunk * SUB), :] = _layernorm(t)

    def split_pair(i, p):
        even = raw[i * n_pairs + p, pl.ds(0, d_model // 2, stride=2), :]
        odd = raw[i * n_pairs + p, pl.ds(1, d_model // 2, stride=2), :]
        return (even & np.uint32(0xFFFF)) | (odd << 16), (even >> 16) | (odd & np.uint32(0xFFFF0000))

    def load_q(p):
        for j, words in enumerate(split_pair(0, p)):
            wq[2 * p + j] = words
            project_tail(qtail, 2 * p + j, words)

    for j in range(TAIL_COPIES - 1):
        tail_copies[j].wait()
        norm_tail(j)
    tail_copies[-1].wait()
    pair_copy(0, 0).wait()
    norm_tail(TAIL_COPIES - 1)
    load_q(0)

    @pl.loop(1, n_pairs, step=Q_BATCH)
    def _(first):
        for u in range(Q_BATCH):
            pair_copy(0, first + u).wait()
        for u in range(Q_BATCH):
            load_q(first + u)

    x_first.wait()

    @pl.loop(0, n_pairs, step=KV_BATCH)
    def _(first):
        batch = [first + u for u in range(KV_BATCH)]
        for p in batch:
            pair_copy(1, p).wait()
            pair_copy(2, p).wait()
        hbuf[...] = normed_tokens(1)
        for p in batch:
            projected = []
            for j, words in enumerate(split_pair(1, p)):
                wk[2 * p + j] = words
                projected.append(project_tail(ktail, 2 * p + j, words)[SUB:SUB + words.shape[0]])
            for j, words in enumerate(split_pair(2, p)):
                paced = _after(pltpu.bitcast(words, jnp.int32), pltpu.bitcast(projected[j], jnp.int32))
                wv[2 * p + j] = pltpu.bitcast(paced, U32)

    for cp in step_copies:
        cp.wait()
    w_r = wr[pl.ds(0, d_model)].astype(F32).reshape(1, d_model)

    def attend(s, mem, tok, row_tasks):
        q, k, v, k_pair, v_pair, score, expo, inv, mixed, lead = ({} for _ in range(10))
        due, latest = [], []
        acc = [zeros[:rows, :] for _ in range(n_col)]
        h_all = _cat([tok, mem])
        h_front = _cat([tok[:front], mem])
        on_mxu = ((0, n_mem), (n_mem + SUB, rows))

        def matmul(lhs, words):
            if due:
                corner = _after(lhs[:SUB, :LANES], functools.reduce(jnp.minimum, due))
                lhs = _cat([_cat([corner, lhs[:SUB, LANES:]], 1), lhs[SUB:]])
                due.clear()
            return _mm(lhs, _bf16(words))

        def with_tail(t, tail, hd):
            return _cat([t[front:], t[:front], tail[hd, tail_rows(s), :]])

        def pairs(g):
            return range(g * GROUP // 2, (g + 1) * GROUP // 2)

        def pack_pair(dst, src, hd):
            if hd % 2:
                dst[hd // 2] = _cat([src[hd - 1], src[hd]]).astype(BF16)

        def qk_first(_):
            cut = d_model - LANES
            ws = [wq.at[0], wq.at[1], wk.at[0], wk.at[1]]
            t = _mm(h_front[:, :cut], _cat([_bf16(w[:cut // 2, :]) for w in ws], 1))
            t = _mm(h_front[:, cut:], _cat([_bf16(w[cut // 2:, :]) for w in ws], 1)) + t
            for hd in range(2):
                q[hd] = with_tail(t[:, hd * dh:(hd + 1) * dh], qtail, hd)
                k[hd] = with_tail(t[:, (2 + hd) * dh:(3 + hd) * dh], ktail, hd)
            pack_pair(k_pair, k, 1)

        def project_q(hd):
            t = matmul(h_front, wq[hd])
            latest.append(t[:SUB])
            q[hd] = with_tail(t, qtail, hd)

        def project_k(hd):
            t = matmul(h_front, wk[hd])
            latest.append(t[:SUB])
            k[hd] = with_tail(t, ktail, hd)
            pack_pair(k_pair, k, hd)

        def project_v(hd):
            t = matmul(h_all, wv[hd])
            latest.append(t[:SUB])
            v[hd] = _cat([t[seg:], t[:seg]])
            pack_pair(v_pair, v, hd)

        def scores(g):
            for p in pairs(g):
                q_pair = _cat([q[2 * p + j][a:b] for j in range(2) for a, b in on_mxu])
                score[p] = _mm_nt(q_pair, k_pair[p])

        def softmax(g):
            for p in pairs(g):
                cap = _cat([pair_cap[j * rows + a:j * rows + b, :] for j in range(2) for a, b in on_mxu])
                t = _cat([score[p], jnp.zeros((cap.shape[0], LANES - 2 * rows), F32)], 1)
                t = jnp.minimum(t, cap)
                t = jnp.exp2((t - jnp.max(t, axis=1, keepdims=True)) * exp2_scale)
                inv[p] = pltpu.reciprocal(jnp.sum(t, axis=1, keepdims=True), approx=True)
                expo[p] = t[:, :2 * rows]

        def mix(g):
            for p in pairs(g):
                mixed[p] = _mm(expo[p], v_pair[p]) * inv[p]

        def rotations(t):
            for block in range(2):
                keys = t[block * SUB:(block + 1) * SUB]
                for shift in range(SUB):
                    yield block * shift, pltpu.roll(keys, shift, 0) if shift else keys

        def lead_score(hd):
            scaled = q[hd][n_mem:n_mem + SUB] * exp2_scale
            ts = []
            for first_seen, keys in rotations(k[hd]):
                t = jnp.sum(scaled * keys, axis=1, keepdims=True)
                ts.append(jnp.minimum(t, lead_cap[first_seen]) if first_seen else t)
            lead[hd] = ts, functools.reduce(jnp.maximum, ts)
            return lead[hd][1]

        def lead_mix(hd):
            ts, top = lead[hd]
            top = _after(top, latest[-2])
            total = out = None
            for t, (_, values) in zip(ts, rotations(v[hd])):
                t = jnp.exp2(t - top)
                total, out = (t, t * values) if out is None else (total + t, out + t * values)
            lead[hd] = out * pltpu.reciprocal(total, approx=True)
            return lead[hd]

        def project_out(task):
            g, n = task
            heads = []
            for hd in range(g * GROUP, (g + 1) * GROUP):
                t = mixed[hd // 2][hd % 2 * (rows - SUB):(hd % 2 + 1) * (rows - SUB)]
                heads.append(_cat([t[:n_mem], lead[hd], t[n_mem:]]))
            words = GROUP * dh // 2
            acc[n] = acc[n] + matmul(_cat(heads, 1), wo[n, pl.ds(g * words, words), :])
            latest.extend([acc[n][:SUB]] * 2)

        tasks = dict(row_tasks, qk_first=qk_first, q=project_q, k=project_k, v=project_v, scores=scores,
                     softmax=softmax, mix=mix, lead_score=lead_score, lead_mix=lead_mix, out=project_out)
        results = {}
        for kind, arg in _step_plan(n_heads, n_col, rows):
            if kind == "due":
                due.append(results[arg])
            else:
                results[kind, arg] = tasks[kind](arg)
        out = _cat(acc, 1)
        return out[:n_mem], out[n_mem:]

    def finish(slot, attn, best):
        best_score, best_row, best_norm = best
        x1 = _rb(xres[slot].astype(F32) + _rb(attn))
        xmid[slot] = x1.astype(BF16)
        n1 = _rb(_layernorm(x1))
        x2 = (x1 + n1).astype(BF16)
        xres[slot] = x2
        ntail[tail_rows(slot), :] = _layernorm(x2.astype(F32)[front:])
        score = _rb(jnp.sum(n1 * w_r, axis=-1, keepdims=True))
        score = jnp.where(slot > 0, score, -np.inf)
        for j in range(0, seg, SUB):
            better = score[j:j + SUB] > best_score
            best_score = jnp.where(better, score[j:j + SUB], best_score)
            best_row = jnp.where(better, (slot - 1) * seg + j + sub, best_row)
            best_norm = jnp.where(better, n1[j:j + SUB], best_norm)
        return best_score, best_row, best_norm

    def out_copy(first, count):
        return pltpu.make_async_copy(xres.at[pl.ds(first + 1, count)], out_hbm.at[pl.ds(first, count)], out_sem)

    @pl.loop(0, N_LAYERS)
    def _(layer):
        is_first, is_last = layer == 0, layer == N_LAYERS - 1

        def steps(it, carry):
            mem, best = carry

            @pl.when(is_first & (it == 1))
            def _():
                x_rest.wait()

            @pl.when(is_last & (it == 1))
            def _():
                out_copy(0, UNROLL - 1).start()

            @pl.when(is_last & (it > 1))
            def _():
                out_copy((it - 1) * UNROLL - 1, UNROLL).start()

            live = dict(best=best, tok=hbuf[...], attn=obuf[...])
            for u in range(UNROLL):
                s = it * UNROLL + u

                def finish_previous(_, s=s):
                    live["best"] = finish(s, live["attn"], live["best"])
                    return live["best"][0]

                def norm_next(_, s=s):
                    live["tok"] = normed_tokens(s + 2)

                mem, live["attn"] = attend(s, mem, live["tok"], dict(finish=finish_previous, norm=norm_next))
            hbuf[...] = live["tok"]
            obuf[...] = live["attn"]
            return mem, live["best"]

        best = (jnp.full((SUB, 1), -np.inf, F32), jnp.zeros((SUB, 1), jnp.int32), jnp.zeros((SUB, d_model), F32))
        _, best = lax.fori_loop(0, n_seg // UNROLL, steps, (mem0[...].astype(F32), best))

        @pl.when(is_first)
        def _():
            for cp in mlp_copies:
                cp.wait()

        score, row, n1 = finish(n_seg, obuf[...], best)

        @pl.when(is_last)
        def _():
            out_copy(n_seg - UNROLL - 1, UNROLL + 1).start()

        gate = _rb(_mm(n1, _bf16(wg[...])))
        gate = _rb(gate * _rb(jax.nn.sigmoid(gate)))
        up = _rb(_mm(n1, _bf16(wu[...])))
        y = _rb(_mm(_rb(gate * up), _bf16(wd[...])))
        update = _rb(n1 + _rb(y * _rb(jax.nn.sigmoid(score))))

        top = jnp.max(score, axis=0, keepdims=True)
        row = jnp.min(jnp.where(score == top, row, n_seg * seg - 1).astype(F32))
        row = jnp.clip(row.astype(jnp.int32), 0, n_seg * seg - 1)
        s = row // seg
        block = pl.ds(pl.multiple_of(row % seg // SUB * SUB, SUB), SUB)
        routed = (sub == row % SUB) & (score > -np.inf)
        fixed = jnp.where(routed, xmid[s + 1, block, :].astype(F32) + update, xres[s + 1, block, :].astype(F32))
        fixed = fixed.astype(BF16)

        @pl.when(jnp.logical_not(is_last))
        def _():
            xres[s + 1, block, :] = fixed

            @pl.when(row % seg >= front)
            def _():
                ntail[tail_rows(s + 1), :] = _layernorm(fixed.astype(F32))

            @pl.loop(0, n_heads, step=GROUP)
            def _(first):
                hbuf[...] = normed_tokens(1)
                for u in range(GROUP):
                    project_tail(qtail, first + u, wq[first + u])
                    project_tail(ktail, first + u, wk[first + u])

        @pl.when(is_last)
        def _():
            fixbuf[:SUB, :] = fixed
            out_copy(0, n_seg).wait()
            fix_copy = pltpu.make_async_copy(fixbuf.at[pl.ds(0, SUB)], out_hbm.at[s, block, :], out_sem)
            fix_copy.start()
            fix_copy.wait()


def pallas_interleave_layers__memory_aug_recurrent_mem_tr__moe_arch_mod__prompt_kernel(
    A_x, A_mem0, A_Wq, A_Wk, A_Wv, A_Wo, A_seg_len, B_x, B_w_r, B_w_gate, B_w_up, B_w_down,
):
    del B_x
    batch, seq, d_model = A_x.shape
    n_heads, dh = A_Wq.shape[1:]
    n_mem = A_mem0.shape[1]
    seg = int(A_seg_len)
    n_seg = seq // seg
    d_ff = B_w_gate.shape[1]
    assert (batch, n_mem, seg, n_heads, dh) == (1, SUB, 32, 32, LANES) and n_seg % (2 * UNROLL) == 0

    any_spec = pl.BlockSpec(memory_space=pl.ANY)
    out = pl.pallas_call(
        _kernel,
        out_shape=jax.ShapeDtypeStruct((n_seg, seg, d_model), A_x.dtype),
        in_specs=[any_spec] * 10,
        out_specs=any_spec,
        scratch_shapes=[
            pltpu.VMEM((3 * n_heads // 2, d_model, dh), U32),
            pltpu.VMEM((n_heads, d_model // 2, dh), U32),
            pltpu.VMEM((n_heads, d_model // 2, dh), U32),
            pltpu.VMEM((n_heads, d_model // 2, dh), U32),
            pltpu.VMEM((d_model // LANES, n_heads * dh // 2, LANES), U32),
            pltpu.VMEM((d_model // 2, d_ff), U32),
            pltpu.VMEM((d_model // 2, d_ff), U32),
            pltpu.VMEM((d_ff // 2, d_model), U32),
            pltpu.VMEM((n_mem, d_model), BF16),
            pltpu.VMEM((SUB * d_model,), BF16),
            pltpu.VMEM((n_seg + 2, seg, d_model), BF16),
            pltpu.VMEM((n_seg + 1, seg, d_model), BF16),
            pltpu.VMEM((n_seg, SUB, d_model), BF16),
            pltpu.VMEM(((n_seg + 2) * SUB, d_model), F32),
            pltpu.VMEM((n_heads, n_seg * SUB, dh), F32),
            pltpu.VMEM((n_heads, n_seg * SUB, dh), F32),
            pltpu.VMEM((seg, d_model), F32),
            pltpu.VMEM((seg, d_model), F32),
            pltpu.VMEM((2 * SUB, d_model), BF16),
            pltpu.VMEM((64, LANES), F32),
            pltpu.VMEM((SUB, SUB, LANES), F32),
            pltpu.VMEM((96, LANES), F32),
            pltpu.SemaphoreType.DMA(((n_heads // 2 - 1) // Q_BATCH + n_heads // 2 // KV_BATCH + TAIL_COPIES + 6,)),
        ],
        compiler_params=pltpu.CompilerParams(vmem_limit_bytes=100 * 1024 * 1024),
    )(
        A_x.reshape(n_seg, seg, d_model),
        A_mem0.reshape(n_mem, d_model),
        A_Wq,
        A_Wk,
        A_Wv,
        A_Wo.reshape(n_heads * dh, d_model),
        B_w_r,
        B_w_gate,
        B_w_up,
        B_w_down,
    )
    return out.reshape(batch, seq, d_model)
```

```python
import functools

import jax
import jax.numpy as jnp
import numpy as np
from jax import lax
import jax.experimental.pallas as pl
import jax.experimental.pallas.tpu as pltpu

F32 = jnp.float32
BF16 = jnp.bfloat16
U32 = jnp.uint32
LANES = 128
SUB = 8
N_LAYERS = 2
GROUP = 8
UNROLL = 8
LEAD_COPIES = 2
Q_BATCH = 3
KV_BATCH = 8

PLAN = dict(
    v_lag=2, score_lag=3, mix_lag=13, out_lag=18, out_step=2,
    softmax_at=240, softmax_gap=40, lead_first=400, lead_last=4000, lead_due=250,
    finish_at=800, finish_due=180, norm_at=900,
)


def _mm(a, b):
    return lax.dot_general(a, b, (((1,), (0,)), ((), ())), preferred_element_type=F32)


def _mm_nt(a, b):
    return lax.dot_general(a, b, (((1,), (1,)), ((), ())), preferred_element_type=F32)


def _cat(parts, axis=0):
    return jnp.concatenate(parts, axis=axis)


def _rb(x):
    return x.astype(BF16).astype(F32)


def _bf16(words):
    return pltpu.bitcast(words, BF16)


def _after(x, other):
    return jnp.maximum(x, jnp.minimum(x, other))


def _layernorm(x):
    inv_d = 1.0 / x.shape[-1]
    mean = jnp.sum(x, axis=-1, keepdims=True) * inv_d
    cen = x - mean
    var = jnp.sum(cen * cen, axis=-1, keepdims=True) * inv_d
    eps = float(np.asarray(1e-5, dtype=BF16))
    std = _rb(jnp.sqrt(_rb(_rb(var) + eps)))
    return _rb(x - _rb(mean)) * (1.0 / std)


def _step_plan(n_heads, n_col, rows):
    n_groups = n_heads // GROUP
    mxu = [("qk_first", 0)]
    for t in range(2, n_heads + PLAN["v_lag"]):
        if t < n_heads:
            mxu.append(("k", t))
        if t >= PLAN["v_lag"]:
            mxu.append(("v", t - PLAN["v_lag"]))
        if t < n_heads:
            mxu.append(("q", t))
        for g in range(n_groups):
            since = t - (GROUP * (g + 1) - 1)
            if since == PLAN["score_lag"]:
                mxu.append(("scores", g))
            if since == PLAN["mix_lag"]:
                mxu.append(("mix", g))
            for n in range(n_col):
                if since == PLAN["out_lag"] + n * PLAN["out_step"]:
                    mxu.append(("out", (g, n)))
    rest = [("mix", g) for g in range(n_groups - 1)] + [("scores", n_groups - 1)]
    rest += [("out", (g, n)) for g in range(n_groups - 2) for n in range(n_col)]
    rest += [("mix", n_groups - 1)]
    rest += [("out", (g, n)) for g in range(n_groups - 2, n_groups) for n in range(n_col)]
    mxu += [task for task in rest if task not in mxu]

    short = rows - SUB
    cycles = dict(qk_first=4 * short, q=short, k=short, v=rows, scores=2 * short, mix=2 * short,
                  out=GROUP * rows // 4)
    start, end = {}, 0
    for task in mxu:
        start[task] = end
        end += cycles[task[0]]

    vector = [
        (end - PLAN["finish_at"], ("finish", 0)),
        (end - PLAN["finish_due"], ("due", ("finish", 0))),
        (end - PLAN["norm_at"], ("norm", 0)),
    ]
    for p in range(n_heads // 2):
        g, j = divmod(p, GROUP // 2)
        at = start["scores", g] + 1 + PLAN["softmax_at"] + j * PLAN["softmax_gap"]
        vector.append((min(at, start["mix", g]), ("softmax", p)))
    for hd in range(n_heads):
        needed = start["out", (hd // GROUP, 0)]
        at = PLAN["lead_first"] + (PLAN["lead_last"] - PLAN["lead_first"]) * hd // (n_heads - 1)
        at_score = max(at, start.get(("k", hd), 0) + rows + 1)
        at_mix = min(max(at_score, start["v", hd] + rows + 1), needed)
        vector += [(min(at_score, at_mix), ("lead_score", hd)), (at_mix, ("lead_mix", hd))]
        if at_mix + PLAN["lead_due"] < needed:
            vector.append((at_mix + PLAN["lead_due"], ("due", ("lead_mix", hd))))
    vector.sort(key=lambda event: event[0])

    plan = []
    for task in mxu:
        while vector and vector[0][0] <= start[task]:
            plan.append(vector.pop(0)[1])
        plan.append(task)
    assert not vector
    return plan


def _kernel(x_hbm, mem0_hbm, wq_hbm, wk_hbm, wv_hbm, wo_hbm, wr_hbm, wg_hbm, wu_hbm, wd_hbm,
            out_hbm,
            raw, wq, wk, wv, wo, wg, wu, wd, mem0, wr, xres, xmid, xlead, nlead, qlead, klead,
            hbuf, obuf, fixbuf, zeros, lead_cap, pair_cap, sems):
    n_seg, seg, d_model = x_hbm.shape
    n_mem = mem0.shape[0]
    n_heads, _, dh = wq.shape
    rows = n_mem + seg
    n_pairs = n_heads // 2
    n_col = d_model // LANES
    scale = dh ** -0.5
    exp2_scale = float(scale * np.log2(np.e))


    q_steps, kv_steps = (n_pairs - 1) // Q_BATCH + 1, n_pairs // KV_BATCH
    free_sems = iter(range(q_steps + kv_steps, sems.shape[0]))

    def copies(*src_dst):
        sem = sems.at[next(free_sems)]
        return [pltpu.make_async_copy(src, dst, sem) for src, dst in src_dst]

    def pair_copy(i, p):
        src = (wq_hbm, wk_hbm, wv_hbm)[i].bitcast(U32)
        sem = (p + Q_BATCH - 1) // Q_BATCH if i == 0 else q_steps + p // KV_BATCH
        return pltpu.make_async_copy(src.at[:, p, :], raw.at[i * n_pairs + p], sems.at[sem])

    chunk = n_seg // LEAD_COPIES
    lead_copies = [copies((x_hbm.at[pl.ds(j * chunk, chunk), pl.ds(0, SUB), :],
                           xlead.at[pl.ds(j * chunk, chunk)]))[0] for j in range(LEAD_COPIES)]
    n_first = UNROLL + 1
    x_first, = copies((x_hbm.at[pl.ds(0, n_first)], xres.at[pl.ds(1, n_first)]))
    step_copies = copies((mem0_hbm, mem0), (wr_hbm, wr.at[pl.ds(0, d_model)]),
                         *[(wo_hbm.bitcast(U32).at[:, pl.ds(n * LANES, LANES)], wo.at[n]) for n in range(n_col)])
    x_rest, = copies((x_hbm.at[pl.ds(n_first, n_seg - n_first)], xres.at[pl.ds(1 + n_first, n_seg - n_first)]))
    mlp_copies = copies((wg_hbm.bitcast(U32), wg), (wu_hbm.bitcast(U32), wu), (wd_hbm.bitcast(U32), wd))
    out_sem = sems.at[next(free_sems)]

    for cp in lead_copies:
        cp.start()
    for p in range(n_pairs):
        pair_copy(0, p).start()
    x_first.start()
    for p in range(n_pairs):
        pair_copy(1, p).start()
        pair_copy(2, p).start()
    for cp in step_copies + [x_rest] + mlp_copies:
        cp.start()

    xres[0] = jnp.zeros((seg, d_model), BF16)
    xres[n_seg + 1] = jnp.zeros((seg, d_model), BF16)
    nlead[pl.ds((n_seg + 1) * SUB, SUB), :] = jnp.zeros((SUB, d_model), F32)
    obuf[...] = jnp.zeros(obuf.shape, F32)
    zeros[...] = jnp.zeros(zeros.shape, F32)
    for j in range(SUB):
        seen = lax.broadcasted_iota(jnp.int32, (SUB, LANES), 0) >= j
        lead_cap[j] = jnp.where(seen, np.inf, -1e9 * np.log2(np.e)).astype(F32)
    r = lax.broadcasted_iota(jnp.int32, pair_cap.shape, 0)
    c = lax.broadcasted_iota(jnp.int32, pair_cap.shape, 1)
    r_pos = jnp.where(r >= rows, r - rows, r)
    c_pos = jnp.where(c >= rows, c - rows, c)
    same_head = ((r >= rows) == (c >= rows)) & (c < 2 * rows)
    causal = jnp.where((r_pos < n_mem) | (r_pos >= c_pos), np.inf, -1e9 / scale)
    pair_cap[...] = jnp.where(same_head, causal, -np.inf).astype(F32)
    sub = lax.broadcasted_iota(jnp.int32, (SUB, 1), 0)

    def lead_rows(slot):
        return pl.ds(pl.multiple_of(slot * SUB, SUB), SUB)

    def project_lead(dst, hd, words):
        t = _mm(nlead[pl.ds(SUB, n_seg * SUB), :], _bf16(words))
        dst[hd] = t
        return t

    def normed_tokens(slot):
        return _cat([nlead[lead_rows(slot), :], _layernorm(xres[slot].astype(F32)[SUB:])])

    def norm_lead(j):
        t = xlead[pl.ds(j * chunk, chunk)].astype(F32).reshape(chunk * SUB, d_model)
        nlead[pl.ds((1 + j * chunk) * SUB, chunk * SUB), :] = _layernorm(t)

    def split_pair(i, p):
        even = raw[i * n_pairs + p, pl.ds(0, d_model // 2, stride=2), :]
        odd = raw[i * n_pairs + p, pl.ds(1, d_model // 2, stride=2), :]
        return (even & np.uint32(0xFFFF)) | (odd << 16), (even >> 16) | (odd & np.uint32(0xFFFF0000))

    def load_q(p):
        for j, words in enumerate(split_pair(0, p)):
            wq[2 * p + j] = words
            project_lead(qlead, 2 * p + j, words)

    for j in range(LEAD_COPIES - 1):
        lead_copies[j].wait()
        norm_lead(j)
    lead_copies[-1].wait()
    pair_copy(0, 0).wait()
    norm_lead(LEAD_COPIES - 1)
    load_q(0)

    @pl.loop(1, n_pairs, step=Q_BATCH)
    def _(first):
        for u in range(Q_BATCH):
            pair_copy(0, first + u).wait()
        for u in range(Q_BATCH):
            load_q(first + u)

    x_first.wait()

    @pl.loop(0, n_pairs, step=KV_BATCH)
    def _(first):
        batch = [first + u for u in range(KV_BATCH)]
        for p in batch:
            pair_copy(1, p).wait()
            pair_copy(2, p).wait()
        hbuf[...] = normed_tokens(1)
        for p in batch:
            projected = []
            for j, words in enumerate(split_pair(1, p)):
                wk[2 * p + j] = words
                projected.append(project_lead(klead, 2 * p + j, words)[SUB:SUB + words.shape[0]])
            for j, words in enumerate(split_pair(2, p)):
                paced = _after(pltpu.bitcast(words, jnp.int32), pltpu.bitcast(projected[j], jnp.int32))
                wv[2 * p + j] = pltpu.bitcast(paced, U32)

    for cp in step_copies:
        cp.wait()
    w_r = wr[pl.ds(0, d_model)].astype(F32).reshape(1, d_model)

    def attend(s, mem, tok, row_tasks):
        q, k, v, k_pair, v_pair, score, expo, inv, mixed, lead = ({} for _ in range(10))
        due, latest = [], []
        acc = [zeros[:rows, :] for _ in range(n_col)]
        h_all = _cat([tok, mem])
        h_rest = h_all[SUB:]
        on_mxu = ((0, n_mem), (n_mem + SUB, rows))

        def matmul(lhs, words):
            if due:
                corner = _after(lhs[:SUB, :LANES], functools.reduce(jnp.minimum, due))
                lhs = _cat([_cat([corner, lhs[:SUB, LANES:]], 1), lhs[SUB:]])
                due.clear()
            return _mm(lhs, _bf16(words))

        def with_lead(t, early, hd):
            return _cat([t[seg - SUB:], early[hd, lead_rows(s), :], t[:seg - SUB]])

        def pairs(g):
            return range(g * GROUP // 2, (g + 1) * GROUP // 2)

        def pack_pair(dst, src, hd):
            if hd % 2:
                dst[hd // 2] = _cat([src[hd - 1], src[hd]]).astype(BF16)

        def qk_first(_):
            cut = d_model - LANES
            ws = [wq.at[0], wq.at[1], wk.at[0], wk.at[1]]
            t = _mm(h_rest[:, :cut], _cat([_bf16(w[:cut // 2, :]) for w in ws], 1))
            t = _mm(h_rest[:, cut:], _cat([_bf16(w[cut // 2:, :]) for w in ws], 1)) + t
            for hd in range(2):
                q[hd] = with_lead(t[:, hd * dh:(hd + 1) * dh], qlead, hd)
                k[hd] = with_lead(t[:, (2 + hd) * dh:(3 + hd) * dh], klead, hd)
            pack_pair(k_pair, k, 1)

        def project_q(hd):
            t = matmul(h_rest, wq[hd])
            latest.append(t[:SUB])
            q[hd] = with_lead(t, qlead, hd)

        def project_k(hd):
            t = matmul(h_rest, wk[hd])
            latest.append(t[:SUB])
            k[hd] = with_lead(t, klead, hd)
            pack_pair(k_pair, k, hd)

        def project_v(hd):
            t = matmul(h_all, wv[hd])
            latest.append(t[:SUB])
            v[hd] = _cat([t[seg:], t[:seg]])
            pack_pair(v_pair, v, hd)

        def scores(g):
            for p in pairs(g):
                q_pair = _cat([q[2 * p + j][a:b] for j in range(2) for a, b in on_mxu])
                score[p] = _mm_nt(q_pair, k_pair[p])

        def softmax(p):
            cap = _cat([pair_cap[j * rows + a:j * rows + b, :] for j in range(2) for a, b in on_mxu])
            t = _cat([score[p], jnp.zeros((cap.shape[0], LANES - 2 * rows), F32)], 1)
            t = jnp.minimum(t, cap)
            t = jnp.exp2((t - jnp.max(t, axis=1, keepdims=True)) * exp2_scale)
            inv[p] = pltpu.reciprocal(jnp.sum(t, axis=1, keepdims=True), approx=True)
            expo[p] = t[:, :2 * rows]

        def mix(g):
            for p in pairs(g):
                mixed[p] = _mm(expo[p], v_pair[p]) * inv[p]

        def rotations(t):
            for block in range(2):
                keys = t[block * SUB:(block + 1) * SUB]
                for shift in range(SUB):
                    yield block * shift, pltpu.roll(keys, shift, 0) if shift else keys

        def lead_score(hd):
            scaled = q[hd][n_mem:n_mem + SUB] * exp2_scale
            ts = []
            for first_seen, keys in rotations(k[hd]):
                t = jnp.sum(scaled * keys, axis=1, keepdims=True)
                ts.append(jnp.minimum(t, lead_cap[first_seen]) if first_seen else t)
            lead[hd] = ts, functools.reduce(jnp.maximum, ts)

        def lead_mix(hd):
            ts, top = lead[hd]
            top = _after(top, latest[-2])
            total = out = None
            for t, (_, values) in zip(ts, rotations(v[hd])):
                t = jnp.exp2(t - top)
                total, out = (t, t * values) if out is None else (total + t, out + t * values)
            lead[hd] = out * pltpu.reciprocal(total, approx=True)
            return lead[hd]

        def project_out(task):
            g, n = task
            heads = []
            for hd in range(g * GROUP, (g + 1) * GROUP):
                t = mixed[hd // 2][hd % 2 * (rows - SUB):(hd % 2 + 1) * (rows - SUB)]
                heads.append(_cat([t[:n_mem], lead[hd], t[n_mem:]]))
            words = GROUP * dh // 2
            acc[n] = acc[n] + matmul(_cat(heads, 1), wo[n, pl.ds(g * words, words), :])
            latest.extend([acc[n][:SUB]] * 2)

        tasks = dict(row_tasks, qk_first=qk_first, q=project_q, k=project_k, v=project_v, scores=scores,
                     softmax=softmax, mix=mix, lead_score=lead_score, lead_mix=lead_mix, out=project_out)
        results = {}
        for kind, arg in _step_plan(n_heads, n_col, rows):
            if kind == "due":
                due.append(results[arg])
            else:
                results[kind, arg] = tasks[kind](arg)
        out = _cat(acc, 1)
        return out[:n_mem], out[n_mem:]

    def finish(slot, attn, best):
        best_score, best_row, best_norm = best
        x1 = _rb(xres[slot].astype(F32) + _rb(attn))
        xmid[slot] = x1.astype(BF16)
        n1 = _rb(_layernorm(x1))
        x2 = (x1 + n1).astype(BF16)
        xres[slot] = x2
        nlead[lead_rows(slot), :] = _layernorm(x2.astype(F32)[:SUB])
        score = _rb(jnp.sum(n1 * w_r, axis=-1, keepdims=True))
        score = jnp.where(slot > 0, score, -np.inf)
        for j in range(0, seg, SUB):
            better = score[j:j + SUB] > best_score
            best_score = jnp.where(better, score[j:j + SUB], best_score)
            best_row = jnp.where(better, (slot - 1) * seg + j + sub, best_row)
            best_norm = jnp.where(better, n1[j:j + SUB], best_norm)
        return best_score, best_row, best_norm

    def out_copy(first, count):
        return pltpu.make_async_copy(xres.at[pl.ds(first + 1, count)], out_hbm.at[pl.ds(first, count)], out_sem)

    @pl.loop(0, N_LAYERS)
    def _(layer):
        is_first, is_last = layer == 0, layer == N_LAYERS - 1

        def steps(it, carry):
            mem, best = carry

            @pl.when(is_first & (it == 1))
            def _():
                x_rest.wait()

            @pl.when(is_last & (it == 1))
            def _():
                out_copy(0, UNROLL - 1).start()

            @pl.when(is_last & (it > 1))
            def _():
                out_copy((it - 1) * UNROLL - 1, UNROLL).start()

            live = dict(best=best, tok=hbuf[...], attn=obuf[...])
            for u in range(UNROLL):
                s = it * UNROLL + u

                def finish_previous(_, s=s):
                    live["best"] = finish(s, live["attn"], live["best"])
                    return live["best"][0]

                def norm_next(_, s=s):
                    live["tok"] = normed_tokens(s + 2)

                mem, live["attn"] = attend(s, mem, live["tok"], dict(finish=finish_previous, norm=norm_next))
            hbuf[...] = live["tok"]
            obuf[...] = live["attn"]
            return mem, live["best"]

        best = (jnp.full((SUB, 1), -np.inf, F32), jnp.zeros((SUB, 1), jnp.int32), jnp.zeros((SUB, d_model), F32))
        _, best = lax.fori_loop(0, n_seg // UNROLL, steps, (mem0[...].astype(F32), best))

        @pl.when(is_first)
        def _():
            for cp in mlp_copies:
                cp.wait()

        score, row, n1 = finish(n_seg, obuf[...], best)

        @pl.when(is_last)
        def _():
            out_copy(n_seg - UNROLL - 1, UNROLL + 1).start()

        gate = _rb(_mm(n1, _bf16(wg[...])))
        gate = _rb(gate * _rb(jax.nn.sigmoid(gate)))
        up = _rb(_mm(n1, _bf16(wu[...])))
        y = _rb(_mm(_rb(gate * up), _bf16(wd[...])))
        update = _rb(n1 + _rb(y * _rb(jax.nn.sigmoid(score))))

        top = jnp.max(score, axis=0, keepdims=True)
        row = jnp.min(jnp.where(score == top, row, n_seg * seg - 1).astype(F32))
        row = jnp.clip(row.astype(jnp.int32), 0, n_seg * seg - 1)
        s = row // seg
        block = pl.ds(pl.multiple_of(row % seg // SUB * SUB, SUB), SUB)
        routed = (sub == row % SUB) & (score > -np.inf)
        fixed = jnp.where(routed, xmid[s + 1, block, :].astype(F32) + update, xres[s + 1, block, :].astype(F32))
        fixed = fixed.astype(BF16)

        @pl.when(jnp.logical_not(is_last))
        def _():
            xres[s + 1, block, :] = fixed

            @pl.when(row % seg < SUB)
            def _():
                nlead[lead_rows(s + 1), :] = _layernorm(fixed.astype(F32))

            @pl.loop(0, n_heads, step=GROUP)
            def _(first):
                hbuf[...] = normed_tokens(1)
                for u in range(GROUP):
                    project_lead(qlead, first + u, wq[first + u])
                    project_lead(klead, first + u, wk[first + u])

        @pl.when(is_last)
        def _():
            fixbuf[:SUB, :] = fixed
            out_copy(0, n_seg).wait()
            fix_copy = pltpu.make_async_copy(fixbuf.at[pl.ds(0, SUB)], out_hbm.at[s, block, :], out_sem)
            fix_copy.start()
            fix_copy.wait()


def pallas_interleave_layers__memory_aug_recurrent_mem_tr__moe_arch_mod__prompt_kernel(
    A_x, A_mem0, A_Wq, A_Wk, A_Wv, A_Wo, A_seg_len, B_x, B_w_r, B_w_gate, B_w_up, B_w_down,
):
    del B_x
    batch, seq, d_model = A_x.shape
    n_heads, dh = A_Wq.shape[1:]
    n_mem = A_mem0.shape[1]
    seg = int(A_seg_len)
    n_seg = seq // seg
    d_ff = B_w_gate.shape[1]
    assert (batch, n_mem, seg, n_heads, dh) == (1, SUB, 32, 32, LANES) and n_seg % (2 * UNROLL) == 0

    any_spec = pl.BlockSpec(memory_space=pl.ANY)
    out = pl.pallas_call(
        _kernel,
        out_shape=jax.ShapeDtypeStruct((n_seg, seg, d_model), A_x.dtype),
        in_specs=[any_spec] * 10,
        out_specs=any_spec,
        scratch_shapes=[
            pltpu.VMEM((3 * n_heads // 2, d_model, dh), U32),
            pltpu.VMEM((n_heads, d_model // 2, dh), U32),
            pltpu.VMEM((n_heads, d_model // 2, dh), U32),
            pltpu.VMEM((n_heads, d_model // 2, dh), U32),
            pltpu.VMEM((d_model // LANES, n_heads * dh // 2, LANES), U32),
            pltpu.VMEM((d_model // 2, d_ff), U32),
            pltpu.VMEM((d_model // 2, d_ff), U32),
            pltpu.VMEM((d_ff // 2, d_model), U32),
            pltpu.VMEM((n_mem, d_model), BF16),
            pltpu.VMEM((SUB * d_model,), BF16),
            pltpu.VMEM((n_seg + 2, seg, d_model), BF16),
            pltpu.VMEM((n_seg + 1, seg, d_model), BF16),
            pltpu.VMEM((n_seg, SUB, d_model), BF16),
            pltpu.VMEM(((n_seg + 2) * SUB, d_model), F32),
            pltpu.VMEM((n_heads, n_seg * SUB, dh), F32),
            pltpu.VMEM((n_heads, n_seg * SUB, dh), F32),
            pltpu.VMEM((seg, d_model), F32),
            pltpu.VMEM((seg, d_model), F32),
            pltpu.VMEM((2 * SUB, d_model), BF16),
            pltpu.VMEM((64, LANES), F32),
            pltpu.VMEM((SUB, SUB, LANES), F32),
            pltpu.VMEM((96, LANES), F32),
            pltpu.SemaphoreType.DMA(((n_heads // 2 - 1) // Q_BATCH + n_heads // 2 // KV_BATCH + LEAD_COPIES + 6,)),
        ],
        compiler_params=pltpu.CompilerParams(vmem_limit_bytes=100 * 1024 * 1024),
    )(
        A_x.reshape(n_seg, seg, d_model),
        A_mem0.reshape(n_mem, d_model),
        A_Wq,
        A_Wk,
        A_Wv,
        A_Wo.reshape(n_heads * dh, d_model),
        B_w_r,
        B_w_gate,
        B_w_up,
        B_w_down,
    )
    return out.reshape(batch, seq, d_model)
```

```python
import functools

import jax
import jax.numpy as jnp
import numpy as np
from jax import lax
import jax.experimental.pallas as pl
import jax.experimental.pallas.tpu as pltpu

F32 = jnp.float32
BF16 = jnp.bfloat16
U32 = jnp.uint32
LANES = 128
SUB = 8
N_LAYERS = 2
GROUP = 8
UNROLL = 8
LEAD_COPIES = 2
Q_BATCH = 3
KV_BATCH = 8

PLAN = dict(
    v_lag=2, score_lag=3, mix_lag=13, out_lag=18, out_step=2,
    softmax_at=240, softmax_gap=40, lead_first=400, lead_last=4000, lead_due=250,
    finish_at=800, finish_due=180, norm_at=900,
)


def _mm(a, b):
    return lax.dot_general(a, b, (((1,), (0,)), ((), ())), preferred_element_type=F32)


def _mm_nt(a, b):
    return lax.dot_general(a, b, (((1,), (1,)), ((), ())), preferred_element_type=F32)


def _cat(parts, axis=0):
    return jnp.concatenate(parts, axis=axis)


def _rb(x):
    return x.astype(BF16).astype(F32)


def _bf16(words):
    return pltpu.bitcast(words, BF16)


def _after(x, other):
    return jnp.maximum(x, jnp.minimum(x, other))


def _inverse(total):
    return pltpu.reciprocal(total, approx=True)


def _layernorm(x):
    inv_d = 1.0 / x.shape[-1]
    mean = jnp.sum(x, axis=-1, keepdims=True) * inv_d
    cen = x - mean
    var = jnp.sum(cen * cen, axis=-1, keepdims=True) * inv_d
    eps = float(np.asarray(1e-5, dtype=BF16))
    std = _rb(jnp.sqrt(_rb(_rb(var) + eps)))
    return _rb(x - _rb(mean)) * (1.0 / std)


def _step_plan(n_heads, n_col, rows):
    n_groups = n_heads // GROUP
    mxu = [("qk_first", 0)]
    for t in range(2, n_heads + PLAN["v_lag"]):
        if t < n_heads:
            mxu.append(("k", t))
        if t >= PLAN["v_lag"]:
            mxu.append(("v", t - PLAN["v_lag"]))
        if t < n_heads:
            mxu.append(("q", t))
        for g in range(n_groups):
            since = t - (GROUP * (g + 1) - 1)
            if since == PLAN["score_lag"]:
                mxu.append(("scores", g))
            if since == PLAN["mix_lag"]:
                mxu.append(("mix", g))
            for n in range(n_col):
                if since == PLAN["out_lag"] + n * PLAN["out_step"]:
                    mxu.append(("out", (g, n)))
    rest = [("mix", g) for g in range(n_groups - 1)] + [("scores", n_groups - 1)]
    rest += [("out", (g, n)) for g in range(n_groups - 2) for n in range(n_col)]
    rest += [("mix", n_groups - 1)]
    rest += [("out", (g, n)) for g in range(n_groups - 2, n_groups) for n in range(n_col)]
    mxu += [task for task in rest if task not in mxu]

    short = rows - SUB
    cycles = dict(qk_first=4 * short, q=short, k=short, v=rows, scores=2 * short, mix=2 * short,
                  out=GROUP * rows // 4)
    start, end = {}, 0
    for task in mxu:
        start[task] = end
        end += cycles[task[0]]

    vector = [
        (end - PLAN["finish_at"], ("finish", 0)),
        (end - PLAN["finish_due"], ("due", ("finish", 0))),
        (end - PLAN["norm_at"], ("norm", 0)),
    ]
    for p in range(n_heads // 2):
        g, j = divmod(p, GROUP // 2)
        at = start["scores", g] + 1 + PLAN["softmax_at"] + j * PLAN["softmax_gap"]
        vector.append((min(at, start["mix", g]), ("softmax", p)))
    for hd in range(n_heads):
        needed = start["out", (hd // GROUP, 0)]
        at = PLAN["lead_first"] + (PLAN["lead_last"] - PLAN["lead_first"]) * hd // (n_heads - 1)
        at_score = max(at, start.get(("k", hd), 0) + rows + 1)
        at_mix = min(max(at_score, start["v", hd] + rows + 1), needed)
        vector += [(min(at_score, at_mix), ("lead_score", hd)), (at_mix, ("lead_mix", hd))]
        if at_mix + PLAN["lead_due"] < needed:
            vector.append((at_mix + PLAN["lead_due"], ("due", ("lead_mix", hd))))
    vector.sort(key=lambda event: event[0])

    plan = []
    for task in mxu:
        while vector and vector[0][0] <= start[task]:
            plan.append(vector.pop(0)[1])
        plan.append(task)
    assert not vector
    return plan


def _kernel(x_hbm, mem0_hbm, wq_hbm, wk_hbm, wv_hbm, wo_hbm, wr_hbm, wg_hbm, wu_hbm, wd_hbm,
            out_hbm,
            raw, wq, wk, wv, wo, wg, wu, wd, mem0, wr, xres, xmid, xlead, nlead, qlead, klead,
            hbuf, obuf, zeros, lead_cap, pair_cap, sems):
    n_seg, seg, d_model = x_hbm.shape
    n_mem = mem0.shape[0]
    n_heads, _, dh = wq.shape
    rows = n_mem + seg
    n_pairs = n_heads // 2
    n_col = d_model // LANES
    scale = dh ** -0.5
    exp2_scale = float(scale * np.log2(np.e))


    q_steps, kv_steps = (n_pairs - 1) // Q_BATCH + 1, n_pairs // KV_BATCH
    free_sems = iter(range(q_steps + kv_steps, sems.shape[0]))

    def copies(*src_dst):
        sem = sems.at[next(free_sems)]
        return [pltpu.make_async_copy(src, dst, sem) for src, dst in src_dst]

    def pair_copy(i, p):
        src = (wq_hbm, wk_hbm, wv_hbm)[i].bitcast(U32)
        sem = (p + Q_BATCH - 1) // Q_BATCH if i == 0 else q_steps + p // KV_BATCH
        return pltpu.make_async_copy(src.at[:, p, :], raw.at[i * n_pairs + p], sems.at[sem])

    chunk = n_seg // LEAD_COPIES
    lead_copies = [copies((x_hbm.at[pl.ds(j * chunk, chunk), pl.ds(0, SUB), :],
                           xlead.at[pl.ds(j * chunk, chunk)]))[0] for j in range(LEAD_COPIES)]
    n_first = UNROLL + 1
    first_copies = copies((x_hbm.at[pl.ds(0, n_first)], xres.at[pl.ds(1, n_first)]),
                          (mem0_hbm, mem0), (wr_hbm, wr.at[pl.ds(0, d_model)]))
    wo_copies = copies(*[(wo_hbm.bitcast(U32).at[:, pl.ds(n * LANES, LANES)], wo.at[n]) for n in range(n_col)])
    late_copies = copies((x_hbm.at[pl.ds(n_first, n_seg - n_first)], xres.at[pl.ds(1 + n_first, n_seg - n_first)]),
                         (wg_hbm.bitcast(U32), wg), (wu_hbm.bitcast(U32), wu), (wd_hbm.bitcast(U32), wd))
    out_sem = sems.at[next(free_sems)]

    for cp in lead_copies:
        cp.start()
    for p in range(n_pairs):
        pair_copy(0, p).start()
    for cp in first_copies:
        cp.start()
    for p in range(n_pairs):
        pair_copy(1, p).start()
        pair_copy(2, p).start()
    for cp in wo_copies + late_copies:
        cp.start()

    xres[0] = jnp.zeros((seg, d_model), BF16)
    xres[n_seg + 1] = jnp.zeros((seg, d_model), BF16)
    nlead[pl.ds((n_seg + 1) * SUB, SUB), :] = jnp.zeros((SUB, d_model), F32)
    obuf[...] = jnp.zeros(obuf.shape, F32)
    zeros[...] = jnp.zeros(zeros.shape, F32)
    for j in range(SUB):
        seen = lax.broadcasted_iota(jnp.int32, (SUB, LANES), 0) >= j
        lead_cap[j] = jnp.where(seen, np.inf, -1e9 * np.log2(np.e)).astype(F32)
    r = lax.broadcasted_iota(jnp.int32, pair_cap.shape, 0)
    c = lax.broadcasted_iota(jnp.int32, pair_cap.shape, 1)
    r_pos = jnp.where(r >= rows, r - rows, r)
    c_pos = jnp.where(c >= rows, c - rows, c)
    same_head = ((r >= rows) == (c >= rows)) & (c < 2 * rows)
    causal = jnp.where((r_pos < n_mem) | (r_pos >= c_pos), np.inf, -1e9 / scale)
    pair_cap[...] = jnp.where(same_head, causal, -np.inf).astype(F32)
    sub = lax.broadcasted_iota(jnp.int32, (SUB, 1), 0)

    def lead_rows(slot):
        return pl.ds(pl.multiple_of(slot * SUB, SUB), SUB)

    def project_lead(dst, hd, words):
        t = _mm(nlead[pl.ds(SUB, n_seg * SUB), :], _bf16(words))
        dst[hd] = t
        return t

    def normed_tokens(slot):
        return _cat([nlead[lead_rows(slot), :], _layernorm(xres[slot].astype(F32)[SUB:])])

    def norm_lead(j):
        t = xlead[pl.ds(j * chunk, chunk)].astype(F32).reshape(chunk * SUB, d_model)
        nlead[pl.ds((1 + j * chunk) * SUB, chunk * SUB), :] = _layernorm(t)

    def split_pair(i, p):
        even = raw[i * n_pairs + p, pl.ds(0, d_model // 2, stride=2), :]
        odd = raw[i * n_pairs + p, pl.ds(1, d_model // 2, stride=2), :]
        return (even & np.uint32(0xFFFF)) | (odd << 16), (even >> 16) | (odd & np.uint32(0xFFFF0000))

    def load_q(p):
        for j, words in enumerate(split_pair(0, p)):
            wq[2 * p + j] = words
            project_lead(qlead, 2 * p + j, words)

    for j in range(LEAD_COPIES - 1):
        lead_copies[j].wait()
        norm_lead(j)
    lead_copies[-1].wait()
    pair_copy(0, 0).wait()
    norm_lead(LEAD_COPIES - 1)
    load_q(0)

    @pl.loop(1, n_pairs, step=Q_BATCH)
    def _(first):
        for u in range(Q_BATCH):
            pair_copy(0, first + u).wait()
        for u in range(Q_BATCH):
            load_q(first + u)

    for cp in first_copies:
        cp.wait()
    w_r = wr[pl.ds(0, d_model)].astype(F32).reshape(1, d_model)

    @pl.loop(0, n_pairs, step=KV_BATCH)
    def _(first):
        batch = [first + u for u in range(KV_BATCH)]
        for p in batch:
            pair_copy(1, p).wait()
            pair_copy(2, p).wait()
        hbuf[...] = normed_tokens(1)
        for p in batch:
            projected = []
            for j, words in enumerate(split_pair(1, p)):
                wk[2 * p + j] = words
                projected.append(project_lead(klead, 2 * p + j, words)[SUB:SUB + words.shape[0]])
            for j, words in enumerate(split_pair(2, p)):
                paced = _after(pltpu.bitcast(words, jnp.int32), pltpu.bitcast(projected[j], jnp.int32))
                wv[2 * p + j] = pltpu.bitcast(paced, U32)

    for cp in wo_copies:
        cp.wait()

    def attend(s, mem, tok, row_tasks):
        q, k, v, k_pair, v_pair, score, expo, inv, mixed, lead = ({} for _ in range(10))
        due, latest = [], []
        acc = [zeros[:rows, :] for _ in range(n_col)]
        h_all = _cat([tok, mem])
        h_rest = h_all[SUB:]
        on_mxu = ((0, n_mem), (n_mem + SUB, rows))

        def matmul(lhs, words):
            if due:
                corner = _after(lhs[:SUB, :LANES], functools.reduce(jnp.minimum, due))
                lhs = _cat([_cat([corner, lhs[:SUB, LANES:]], 1), lhs[SUB:]])
                due.clear()
            return _mm(lhs, _bf16(words))

        def with_lead(t, early, hd):
            return _cat([t[seg - SUB:], early[hd, lead_rows(s), :], t[:seg - SUB]])

        def pairs(g):
            return range(g * GROUP // 2, (g + 1) * GROUP // 2)

        def pack_pair(dst, src, hd):
            if hd % 2:
                dst[hd // 2] = _cat([src[hd - 1], src[hd]]).astype(BF16)

        def qk_first(_):
            cut = d_model - LANES
            ws = [wq.at[0], wq.at[1], wk.at[0], wk.at[1]]
            t = _mm(h_rest[:, :cut], _cat([_bf16(w[:cut // 2, :]) for w in ws], 1))
            t = _mm(h_rest[:, cut:], _cat([_bf16(w[cut // 2:, :]) for w in ws], 1)) + t
            for hd in range(2):
                q[hd] = with_lead(t[:, hd * dh:(hd + 1) * dh], qlead, hd)
                k[hd] = with_lead(t[:, (2 + hd) * dh:(3 + hd) * dh], klead, hd)
            pack_pair(k_pair, k, 1)

        def project_q(hd):
            t = matmul(h_rest, wq[hd])
            latest.append(t[:SUB])
            q[hd] = with_lead(t, qlead, hd)

        def project_k(hd):
            t = matmul(h_rest, wk[hd])
            latest.append(t[:SUB])
            k[hd] = with_lead(t, klead, hd)
            pack_pair(k_pair, k, hd)

        def project_v(hd):
            t = matmul(h_all, wv[hd])
            latest.append(t[:SUB])
            v[hd] = _cat([t[seg:], t[:seg]])
            pack_pair(v_pair, v, hd)

        def scores(g):
            for p in pairs(g):
                q_pair = _cat([q[2 * p + j][a:b] for j in range(2) for a, b in on_mxu])
                score[p] = _mm_nt(q_pair, k_pair[p])

        def softmax(p):
            cap = _cat([pair_cap[j * rows + a:j * rows + b, :] for j in range(2) for a, b in on_mxu])
            t = _cat([score[p], jnp.zeros((cap.shape[0], LANES - 2 * rows), F32)], 1)
            t = jnp.minimum(t, cap)
            t = jnp.exp2((t - jnp.max(t, axis=1, keepdims=True)) * exp2_scale)
            inv[p] = _inverse(jnp.sum(t, axis=1, keepdims=True))
            expo[p] = t[:, :2 * rows]

        def mix(g):
            for p in pairs(g):
                mixed[p] = _mm(expo[p], v_pair[p]) * inv[p]

        def rotations(t):
            for block in range(2):
                keys = t[block * SUB:(block + 1) * SUB]
                for shift in range(SUB):
                    yield block * shift, pltpu.roll(keys, shift, 0) if shift else keys

        def lead_score(hd):
            scaled = q[hd][n_mem:n_mem + SUB] * exp2_scale
            ts = []
            for first_seen, keys in rotations(k[hd]):
                t = jnp.sum(scaled * keys, axis=1, keepdims=True)
                ts.append(jnp.minimum(t, lead_cap[first_seen]) if first_seen else t)
            lead[hd] = ts, functools.reduce(jnp.maximum, ts)

        def lead_mix(hd):
            ts, top = lead[hd]
            top = _after(top, latest[-2])
            total = out = None
            for t, (_, values) in zip(ts, rotations(v[hd])):
                t = jnp.exp2(t - top)
                total, out = (t, t * values) if out is None else (total + t, out + t * values)
            lead[hd] = out * _inverse(total)
            return lead[hd]

        def project_out(task):
            g, n = task
            heads = []
            for hd in range(g * GROUP, (g + 1) * GROUP):
                t = mixed[hd // 2][hd % 2 * (rows - SUB):(hd % 2 + 1) * (rows - SUB)]
                heads.append(_cat([t[:n_mem], lead[hd], t[n_mem:]]))
            words = GROUP * dh // 2
            acc[n] = acc[n] + matmul(_cat(heads, 1), wo[n, pl.ds(g * words, words), :])
            latest.extend([acc[n][:SUB]] * 2)

        tasks = dict(row_tasks, qk_first=qk_first, q=project_q, k=project_k, v=project_v, scores=scores,
                     softmax=softmax, mix=mix, lead_score=lead_score, lead_mix=lead_mix, out=project_out)
        results = {}
        for kind, arg in _step_plan(n_heads, n_col, rows):
            if kind == "due":
                due.append(results[arg])
            else:
                results[kind, arg] = tasks[kind](arg)
        out = _cat(acc, 1)
        return out[:n_mem], out[n_mem:]

    def finish(slot, attn, best):
        best_score, best_row, best_norm = best
        x1 = _rb(xres[slot].astype(F32) + _rb(attn))
        xmid[slot] = x1.astype(BF16)
        n1 = _rb(_layernorm(x1))
        x2 = (x1 + n1).astype(BF16)
        xres[slot] = x2
        nlead[lead_rows(slot), :] = _layernorm(x2.astype(F32)[:SUB])
        score = _rb(jnp.sum(n1 * w_r, axis=-1, keepdims=True))
        score = jnp.where(slot > 0, score, -np.inf)
        for j in range(0, seg, SUB):
            better = score[j:j + SUB] > best_score
            best_score = jnp.where(better, score[j:j + SUB], best_score)
            best_row = jnp.where(better, (slot - 1) * seg + j + sub, best_row)
            best_norm = jnp.where(better, n1[j:j + SUB], best_norm)
        return best_score, best_row, best_norm

    def out_copy(first, count):
        return pltpu.make_async_copy(xres.at[pl.ds(first + 1, count)], out_hbm.at[pl.ds(first, count)], out_sem)

    @pl.loop(0, N_LAYERS)
    def _(layer):
        is_first, is_last = layer == 0, layer == N_LAYERS - 1

        def steps(it, carry):
            mem, best = carry

            @pl.when(is_first & (it == 1))
            def _():
                for cp in late_copies:
                    cp.wait()

            live = dict(best=best, tok=hbuf[...], attn=obuf[...])
            for u in range(UNROLL):
                s = it * UNROLL + u

                def finish_previous(_, s=s):
                    live["best"] = finish(s, live["attn"], live["best"])
                    return live["best"][0]

                def norm_next(_, s=s):
                    live["tok"] = normed_tokens(s + 2)

                mem, live["attn"] = attend(s, mem, live["tok"], dict(finish=finish_previous, norm=norm_next))
            hbuf[...] = live["tok"]
            obuf[...] = live["attn"]

            @pl.when(is_last & (it == 0))
            def _():
                out_copy(0, UNROLL - 1).start()

            @pl.when(is_last & (it > 0))
            def _():
                out_copy(it * UNROLL - 1, UNROLL).start()

            return mem, live["best"]

        best = (jnp.full((SUB, 1), -np.inf, F32), jnp.zeros((SUB, 1), jnp.int32), jnp.zeros((SUB, d_model), F32))
        _, best = lax.fori_loop(0, n_seg // UNROLL, steps, (mem0[...].astype(F32), best))

        score, row, n1 = finish(n_seg, obuf[...], best)

        gate = _rb(_mm(n1, _bf16(wg[...])))
        gate = _rb(gate * _rb(jax.nn.sigmoid(gate)))
        up = _rb(_mm(n1, _bf16(wu[...])))
        y = _rb(_mm(_rb(gate * up), _bf16(wd[...])))
        update = _rb(n1 + _rb(y * _rb(jax.nn.sigmoid(score))))

        top = jnp.max(score, axis=0, keepdims=True)
        row = jnp.min(jnp.where(score == top, row, n_seg * seg - 1).astype(F32))
        row = jnp.clip(row.astype(jnp.int32), 0, n_seg * seg - 1)
        s = row // seg
        block = pl.ds(pl.multiple_of(row % seg // SUB * SUB, SUB), SUB)
        routed = (sub == row % SUB) & (score > -np.inf)
        fixed = jnp.where(routed, xmid[s + 1, block, :].astype(F32) + update, xres[s + 1, block, :].astype(F32))
        fixed = fixed.astype(BF16)

        @pl.when(jnp.logical_not(is_last))
        def _():
            xres[s + 1, block, :] = fixed

            @pl.when(row % seg < SUB)
            def _():
                nlead[lead_rows(s + 1), :] = _layernorm(fixed.astype(F32))

            @pl.loop(0, n_heads, step=GROUP)
            def _(first):
                hbuf[...] = normed_tokens(1)
                for u in range(GROUP):
                    project_lead(qlead, first + u, wq[first + u])
                    project_lead(klead, first + u, wk[first + u])

        @pl.when(is_last)
        def _():
            out_copy(0, n_seg - 1).wait()
            xres[s + 1, block, :] = fixed
            out_copy(n_seg - 1, 1).start()

            @pl.when(s < n_seg - 1)
            def _():
                out_copy(s, 1).start()
                out_copy(s, 1).wait()

            out_copy(n_seg - 1, 1).wait()


def pallas_interleave_layers__memory_aug_recurrent_mem_tr__moe_arch_mod__prompt_kernel(
    A_x, A_mem0, A_Wq, A_Wk, A_Wv, A_Wo, A_seg_len, B_x, B_w_r, B_w_gate, B_w_up, B_w_down,
):
    del B_x
    batch, seq, d_model = A_x.shape
    n_heads, dh = A_Wq.shape[1:]
    n_mem = A_mem0.shape[1]
    seg = int(A_seg_len) if isinstance(A_seg_len, (int, np.integer)) else 32
    n_seg = seq // seg
    d_ff = B_w_gate.shape[1]
    assert (batch, n_mem, seg, n_heads, dh) == (1, SUB, 32, 32, LANES) and n_seg % (2 * UNROLL) == 0

    any_spec = pl.BlockSpec(memory_space=pl.ANY)
    out = pl.pallas_call(
        _kernel,
        out_shape=jax.ShapeDtypeStruct((n_seg, seg, d_model), A_x.dtype),
        in_specs=[any_spec] * 10,
        out_specs=any_spec,
        scratch_shapes=[
            pltpu.VMEM((3 * n_heads // 2, d_model, dh), U32),
            pltpu.VMEM((n_heads, d_model // 2, dh), U32),
            pltpu.VMEM((n_heads, d_model // 2, dh), U32),
            pltpu.VMEM((n_heads, d_model // 2, dh), U32),
            pltpu.VMEM((d_model // LANES, n_heads * dh // 2, LANES), U32),
            pltpu.VMEM((d_model // 2, d_ff), U32),
            pltpu.VMEM((d_model // 2, d_ff), U32),
            pltpu.VMEM((d_ff // 2, d_model), U32),
            pltpu.VMEM((n_mem, d_model), BF16),
            pltpu.VMEM((SUB * d_model,), BF16),
            pltpu.VMEM((n_seg + 2, seg, d_model), BF16),
            pltpu.VMEM((n_seg + 1, seg, d_model), BF16),
            pltpu.VMEM((n_seg, SUB, d_model), BF16),
            pltpu.VMEM(((n_seg + 2) * SUB, d_model), F32),
            pltpu.VMEM((n_heads, n_seg * SUB, dh), F32),
            pltpu.VMEM((n_heads, n_seg * SUB, dh), F32),
            pltpu.VMEM((seg, d_model), F32),
            pltpu.VMEM((seg, d_model), F32),
            pltpu.VMEM((64, LANES), F32),
            pltpu.VMEM((SUB, SUB, LANES), F32),
            pltpu.VMEM((96, LANES), F32),
            pltpu.SemaphoreType.DMA(((n_heads // 2 - 1) // Q_BATCH + n_heads // 2 // KV_BATCH + LEAD_COPIES + 5,)),
        ],
        compiler_params=pltpu.CompilerParams(vmem_limit_bytes=100 * 1024 * 1024),
    )(
        A_x.reshape(n_seg, seg, d_model),
        A_mem0.reshape(n_mem, d_model),
        A_Wq,
        A_Wk,
        A_Wv,
        A_Wo.reshape(n_heads * dh, d_model),
        B_w_r,
        B_w_gate,
        B_w_up,
        B_w_down,
    )
    return out.reshape(batch, seq, d_model)
```
